```python
import jax
import jax.numpy as jnp

def _softmax(x, axis=-1):
    return jax.nn.softmax(x, axis=axis)

def _gelu(x):
    return jax.nn.gelu(x, approximate=True)

def _silu(x):
    return jax.nn.silu(x)

def _sigmoid(x):
    return jax.nn.sigmoid(x)

def _layernorm(x, axis=-1, eps=1e-05):
    m = jnp.mean(x, axis=axis, keepdims=True)
    v = jnp.var(x, axis=axis, keepdims=True)
    return (x - m) / jnp.sqrt(v + eps)

def _scatter_add(tgt, idx, src, axis=0):
    return tgt.at[idx].add(src)

def _segment_sum(src, seg, n):
    return jax.ops.segment_sum(src, seg, n)

class _Rng:

    def __init__(self, key):
        self._k = key

    def _next(self):
        self._k, sub = jax.random.split(self._k)
        return sub

    def normal(self, shape):
        return jax.random.normal(self._next(), shape, dtype=jnp.bfloat16)

    def randint(self, lo, hi, shape):
        return jax.random.randint(self._next(), shape, lo, hi, dtype=jnp.int32)

    def uniform(self, shape, lo=0.0, hi=1.0):
        return jax.random.uniform(self._next(), shape, jnp.bfloat16, lo, hi)

    def permutation(self, n):
        return jax.random.permutation(self._next(), n)
kernel_name = 'recurrent_scan__memory_aug_recurrent_mem_tr__glu_gated_glu__prompt'

def setup_inputs():
    _rng = _Rng(jax.random.key(int.from_bytes(__import__("os").urandom(4), "little")))
    _w = lambda a: (lambda t: t.astype(jnp.bfloat16) if jnp.issubdtype(t.dtype, jnp.floating) else t)(jnp.asarray(a))

    def _A_setup():
        B, S, Dm = (1, 2048, 1024)
        H, Dh = (32, 128)
        M, seg = (8, 32)
        seg = min(seg, S)
        S = S // seg * seg
        return {'x': _w((lambda *s: _rng.normal(s) * 0.05)(B, S, Dm)), 'mem0': _w((lambda *s: _rng.normal(s) * 0.05)(B, M, Dm)), 'Wq': _w((lambda *s: _rng.normal(s) * 0.05)(Dm, H, Dh) * Dm ** (-0.5)), 'Wk': _w((lambda *s: _rng.normal(s) * 0.05)(Dm, H, Dh) * Dm ** (-0.5)), 'Wv': _w((lambda *s: _rng.normal(s) * 0.05)(Dm, H, Dh) * Dm ** (-0.5)), 'Wo': _w((lambda *s: _rng.normal(s) * 0.05)(H, Dh, Dm) * (H * Dh) ** (-0.5)), 'seg_len': seg}
    _A_in = _A_setup()

    def _B_setup():
        B, S, D, F = (1, 2048, 1024, 3584)
        return {'x': _w((lambda *s: _rng.normal(s) * 0.05)(B, S, D)), 'w_gate': _w((lambda *s: _rng.normal(s) * 0.05)(D, F)), 'w_up': _w((lambda *s: _rng.normal(s) * 0.05)(D, F)), 'w_down': _w((lambda *s: _rng.normal(s) * 0.05)(F, D))}
    _B_in = _B_setup()
    return {'A_x': _A_in['x'], 'A_mem0': _A_in['mem0'], 'A_Wq': _A_in['Wq'], 'A_Wk': _A_in['Wk'], 'A_Wv': _A_in['Wv'], 'A_Wo': _A_in['Wo'], 'A_seg_len': _A_in['seg_len'], 'B_x': _B_in['x'], 'B_w_gate': _B_in['w_gate'], 'B_w_up': _B_in['w_up'], 'B_w_down': _B_in['w_down']}

def reference(A_x, A_mem0, A_Wq, A_Wk, A_Wv, A_Wo, A_seg_len, B_x, B_w_gate, B_w_up, B_w_down):

    def _A_ref(x, mem0, Wq, Wk, Wv, Wo, seg_len):
        B, S, Dm = x.shape
        H, Dh = (Wq.shape[1], Wq.shape[2])
        M = mem0.shape[1]
        scale = Dh ** (-0.5)
        n_seg = S // seg_len
        L = M + seg_len
        idx = jnp.arange(L)
        mask = (idx[:, None] < M) | (idx[:, None] >= idx[None, :])
        mem = mem0
        outs = []
        for s in range(n_seg):
            xs = x[:, s * seg_len:(s + 1) * seg_len, :].copy()
            h = jnp.concatenate([mem, xs], axis=1)
            q = jnp.einsum('btd,dhe->bhte', h, Wq)
            k = jnp.einsum('btd,dhe->bhte', h, Wk)
            v = jnp.einsum('btd,dhe->bhte', h, Wv)
            scores = jnp.einsum('bhqe,bhke->bhqk', q, k) * scale
            scores = jnp.where(mask[None, None], scores, -1000000000.0)
            p = _softmax(scores, axis=-1)
            o = jnp.einsum('bhqk,bhke->bhqe', p, v)
            o = jnp.einsum('bhte,hed->btd', o, Wo)
            mem = o[:, :M, :].copy()
            outs.append(o[:, M:, :])
        return jnp.concatenate(outs, axis=1)

    def _B_ref(x, w_gate, w_up, w_down):
        g = jnp.einsum('bsd,df->bsf', x, w_gate)
        u = jnp.einsum('bsd,df->bsf', x, w_up)
        h = _sigmoid(g) * u
        return jnp.einsum('bsf,fd->bsd', h, w_down)
    x = A_x
    xn = _layernorm(x, axis=-1)
    s = _A_ref(xn, A_mem0, A_Wq, A_Wk, A_Wv, A_Wo, A_seg_len)
    g = _silu(_B_ref(xn, B_w_gate, B_w_up, B_w_down))
    return x + s * g
```

```python
import functools

import jax
import jax.numpy as jnp
import numpy as np
import jax.experimental.pallas as pl
import jax.experimental.pallas.tpu as pltpu

_F32 = jnp.float32
_BF16 = jnp.bfloat16
_U32 = jnp.uint32


def _as_bf16(w_u32):
    return pltpu.bitcast(w_u32, _BF16)


def _kernel(x_hbm, mem0_ref, wq_hbm, wk_hbm, wv_hbm, wo_hbm, wg_hbm, wu_hbm, wd_hbm,
            out_hbm,
            x_v, xn_v, gate_v, out_v, wq_v, wk_v, wv_v, wo_v, wg_v, wu_v, wd_v, st_v,
            sems,
            *, S, D, H, E, M, SEG, F, MB, FC, HG):
    n_seg = S // SEG
    scale = E ** (-0.5)
    L = M + SEG

    cp_x = pltpu.make_async_copy(x_hbm, x_v, sems.at[0])
    cp_g = pltpu.make_async_copy(wg_hbm.bitcast(_U32), wg_v, sems.at[1])
    cp_u = pltpu.make_async_copy(wu_hbm.bitcast(_U32), wu_v, sems.at[2])
    cp_d = pltpu.make_async_copy(wd_hbm.bitcast(_U32), wd_v, sems.at[3])
    cp_o = pltpu.make_async_copy(wo_hbm.bitcast(_U32), wo_v, sems.at[4])

    def gather_copies(w_hbm, slot):
        wu = w_hbm.bitcast(_U32)
        return [pltpu.make_async_copy(wu.at[:, p, h2, :], st_v.at[slot, p, h2], sems.at[5 + slot])
                for p in range(2) for h2 in range(H // 2)]

    def repack(slot, dst):
        @pl.loop(0, H // 2)
        def _(h2):
            a = st_v[slot, 0, h2]
            b = st_v[slot, 1, h2]
            lo = (a & 0xFFFF) | (b << 16)
            hi = (a >> 16) | (b & np.uint32(0xFFFF0000))
            c0 = pl.multiple_of(h2 * (2 * E), 2 * E)
            dst[:, pl.ds(c0, E)] = lo
            dst[:, pl.ds(c0 + E, E)] = hi

    cp_x.start()
    cp_g.start()
    cp_u.start()
    cp_d.start()
    cp_o.start()
    for c in gather_copies(wq_hbm, 0):
        c.start()
    for c in gather_copies(wk_hbm, 1):
        c.start()

    cp_x.wait()

    @pl.loop(0, S // 64)
    def _(i):
        r = pl.multiple_of(i * 64, 64)
        xv = x_v[pl.ds(r, 64), :].astype(_F32)
        mu = jnp.mean(xv, axis=-1, keepdims=True)
        xc = xv - mu
        var = jnp.mean(xc * xc, axis=-1, keepdims=True)
        xn_v[pl.ds(r, 64), :] = xc / jnp.sqrt(var + 1e-5)

    cp_g.wait()
    cp_u.wait()
    cp_d.wait()

    @pl.loop(0, S // MB)
    def _(i):
        r = pl.multiple_of(i * MB, MB)
        xb = xn_v[pl.ds(r, MB), :].astype(_BF16)
        acc = None
        for c in range(F // FC):
            g = jnp.dot(xb, _as_bf16(wg_v[:, c * FC:(c + 1) * FC]), preferred_element_type=_F32)
            u = jnp.dot(xb, _as_bf16(wu_v[:, c * FC:(c + 1) * FC]), preferred_element_type=_F32)
            hh = (jax.nn.sigmoid(g) * u).astype(_BF16)
            d = jnp.dot(hh, _as_bf16(wd_v[c * (FC // 2):(c + 1) * (FC // 2), :]),
                        preferred_element_type=_F32)
            acc = d if acc is None else acc + d
        gate_v[pl.ds(r, MB), :] = jax.nn.silu(acc)

    for c in gather_copies(wq_hbm, 0):
        c.wait()
    repack(0, wq_v)
    for c in gather_copies(wv_hbm, 0):
        c.start()
    for c in gather_copies(wk_hbm, 1):
        c.wait()
    repack(1, wk_v)
    for c in gather_copies(wv_hbm, 0):
        c.wait()
    repack(0, wv_v)
    cp_o.wait()

    row = jax.lax.broadcasted_iota(jnp.int32, (L, L), 0)
    col = jax.lax.broadcasted_iota(jnp.int32, (L, L), 1)
    mask = (row < M) | (row >= col)
    GW = HG * E

    def step(s, mem):
        r = pl.multiple_of(s * SEG, SEG)
        hb = jnp.concatenate([mem, xn_v[pl.ds(r, SEG), :]], axis=0).astype(_BF16)

        def qkv(g):
            return tuple(
                jnp.dot(hb, _as_bf16(w[:, g * GW:(g + 1) * GW]), preferred_element_type=_F32).astype(_BF16)
                for w in (wq_v, wk_v, wv_v))

        def attn(t):
            q, k, v = t
            outs = []
            for j in range(HG):
                sl = slice(j * E, (j + 1) * E)
                sc = jax.lax.dot_general(q[:, sl], k[:, sl], (((1,), (1,)), ((), ())),
                                         preferred_element_type=_F32) * scale
                sc = jnp.where(mask, sc, -1e9)
                mx = jnp.max(sc, axis=-1, keepdims=True)
                e = jnp.exp(sc - mx)
                p = e / jnp.sum(e, axis=-1, keepdims=True)
                outs.append(jnp.dot(p.astype(_BF16), v[:, sl], preferred_element_type=_F32).astype(_BF16))
            return jnp.concatenate(outs, axis=1)

        def proj(g, o):
            return jnp.dot(o, _as_bf16(wo_v[g * (GW // 2):(g + 1) * (GW // 2), :]),
                           preferred_element_type=_F32)

        n_g = H // HG
        res = None
        cur = qkv(0)
        for g in range(n_g):
            nxt = qkv(g + 1) if g + 1 < n_g else None
            d = proj(g, attn(cur))
            res = d if res is None else res + d
            cur = nxt
        xr = x_v[pl.ds(r, SEG), :].astype(_F32)
        out_v[pl.ds(r, SEG), :] = (xr + res[M:] * gate_v[pl.ds(r, SEG), :]).astype(out_v.dtype)
        return res[:M]

    jax.lax.fori_loop(0, n_seg, step, mem0_ref[...].astype(_F32))

    cp_out = pltpu.make_async_copy(out_v, out_hbm, sems.at[0])
    cp_out.start()
    cp_out.wait()


@functools.partial(jax.jit, static_argnames=("A_seg_len",))
def pallas_recurrent_scan__memory_aug_recurrent_mem_tr__glu_gated_glu__prompt_kernel(
    A_x: jax.Array,
    A_mem0: jax.Array,
    A_Wq: jax.Array,
    A_Wk: jax.Array,
    A_Wv: jax.Array,
    A_Wo: jax.Array,
    A_seg_len: int,
    B_x: jax.Array,
    B_w_gate: jax.Array,
    B_w_up: jax.Array,
    B_w_down: jax.Array,
):
    del B_x
    B, S, D = A_x.shape
    _, H, E = A_Wq.shape
    M = A_mem0.shape[1]
    F = B_w_gate.shape[1]
    SEG = int(A_seg_len)
    assert B == 1 and S % SEG == 0

    kern = functools.partial(_kernel, S=S, D=D, H=H, E=E, M=M, SEG=SEG, F=F, MB=256, FC=512, HG=4)
    any_spec = pl.BlockSpec(memory_space=pl.ANY)
    out = pl.pallas_call(
        kern,
        out_shape=jax.ShapeDtypeStruct((S, D), A_x.dtype),
        in_specs=[any_spec, pl.BlockSpec(memory_space=pltpu.VMEM)] + [any_spec] * 7,
        out_specs=any_spec,
        scratch_shapes=[
            pltpu.VMEM((S, D), _BF16),
            pltpu.VMEM((S, D), _F32),
            pltpu.VMEM((S, D), _F32),
            pltpu.VMEM((S, D), _BF16),
            pltpu.VMEM((D // 2, H * E), _U32),
            pltpu.VMEM((D // 2, H * E), _U32),
            pltpu.VMEM((D // 2, H * E), _U32),
            pltpu.VMEM((H * E // 2, D), _U32),
            pltpu.VMEM((D // 2, F), _U32),
            pltpu.VMEM((D // 2, F), _U32),
            pltpu.VMEM((F // 2, D), _U32),
            pltpu.VMEM((2, 2, H // 2, D // 2, E), _U32),
            pltpu.SemaphoreType.DMA((8,)),
        ],
        compiler_params=pltpu.CompilerParams(vmem_limit_bytes=120 * 1024 * 1024),
    )(
        A_x.reshape(S, D),
        A_mem0.reshape(M, D),
        A_Wq.reshape(D // 2, 2, H, E),
        A_Wk.reshape(D // 2, 2, H, E),
        A_Wv.reshape(D // 2, 2, H, E),
        A_Wo.reshape(H * E, D),
        B_w_gate,
        B_w_up,
        B_w_down,
    )
    return out.reshape(B, S, D)
```

```python
import functools

import jax
import jax.numpy as jnp
import numpy as np
import jax.experimental.pallas as pl
import jax.experimental.pallas.tpu as pltpu

_F32 = jnp.float32
_BF16 = jnp.bfloat16
_U32 = jnp.uint32


def _as_bf16(w_u32):
    return pltpu.bitcast(w_u32, _BF16)


def _kernel(x_hbm, mem0_ref, wq_hbm, wk_hbm, wv_hbm, wo_hbm, wg_hbm, wu_hbm, wd_hbm,
            out_hbm,
            x_v, xn_v, gate_v, out_v, wq_v, wk_v, wv_v, wo_v, wg_v, wu_v, wd_v, st_v,
            sems,
            *, S, D, H, E, M, SEG, F, MB, FC, HG):
    n_seg = S // SEG
    scale = E ** (-0.5)
    L = M + SEG

    cp_x = pltpu.make_async_copy(x_hbm, x_v, sems.at[0])
    cp_g = pltpu.make_async_copy(wg_hbm.bitcast(_U32), wg_v, sems.at[1])
    cp_u = pltpu.make_async_copy(wu_hbm.bitcast(_U32), wu_v, sems.at[2])
    cp_d = pltpu.make_async_copy(wd_hbm.bitcast(_U32), wd_v, sems.at[3])
    cp_o = pltpu.make_async_copy(wo_hbm.bitcast(_U32), wo_v, sems.at[4])

    def gather_copies(w_hbm, slot):
        wu = w_hbm.bitcast(_U32)
        return [pltpu.make_async_copy(wu.at[:, p, h2, :], st_v.at[slot, p, h2], sems.at[5 + slot])
                for p in range(2) for h2 in range(H // 2)]

    def repack(slot, dst):
        @pl.loop(0, H // 2)
        def _(h2):
            a = st_v[slot, 0, h2]
            b = st_v[slot, 1, h2]
            lo = (a & 0xFFFF) | (b << 16)
            hi = (a >> 16) | (b & np.uint32(0xFFFF0000))
            c0 = pl.multiple_of(h2 * (2 * E), 2 * E)
            dst[:, pl.ds(c0, E)] = lo
            dst[:, pl.ds(c0 + E, E)] = hi

    cp_x.start()
    cp_g.start()
    cp_u.start()
    cp_d.start()
    cp_o.start()
    for c in gather_copies(wq_hbm, 0):
        c.start()
    for c in gather_copies(wk_hbm, 1):
        c.start()

    cp_x.wait()

    @pl.loop(0, S // 64)
    def _(i):
        r = pl.multiple_of(i * 64, 64)
        xv = x_v[pl.ds(r, 64), :].astype(_F32)
        mu = jnp.mean(xv, axis=-1, keepdims=True)
        xc = xv - mu
        var = jnp.mean(xc * xc, axis=-1, keepdims=True)
        xn_v[pl.ds(r, 64), :] = xc / jnp.sqrt(var + 1e-5)

    cp_g.wait()
    cp_u.wait()
    cp_d.wait()

    @pl.loop(0, S // MB)
    def _(i):
        r = pl.multiple_of(i * MB, MB)
        xb = xn_v[pl.ds(r, MB), :].astype(_BF16)
        acc = None
        for c in range(F // FC):
            g = jnp.dot(xb, _as_bf16(wg_v[:, c * FC:(c + 1) * FC]), preferred_element_type=_F32)
            u = jnp.dot(xb, _as_bf16(wu_v[:, c * FC:(c + 1) * FC]), preferred_element_type=_F32)
            hh = (jax.nn.sigmoid(g) * u).astype(_BF16)
            d = jnp.dot(hh, _as_bf16(wd_v[c * (FC // 2):(c + 1) * (FC // 2), :]),
                        preferred_element_type=_F32)
            acc = d if acc is None else acc + d
        gate_v[pl.ds(r, MB), :] = jax.nn.silu(acc)

    for c in gather_copies(wq_hbm, 0):
        c.wait()
    repack(0, wq_v)
    for c in gather_copies(wv_hbm, 0):
        c.start()
    for c in gather_copies(wk_hbm, 1):
        c.wait()
    repack(1, wk_v)
    for c in gather_copies(wv_hbm, 0):
        c.wait()
    repack(0, wv_v)
    cp_o.wait()

    row = jax.lax.broadcasted_iota(jnp.int32, (2 * L, 2 * L), 0)
    col = jax.lax.broadcasted_iota(jnp.int32, (2 * L, 2 * L), 1)
    r_in = jnp.where(row >= L, row - L, row)
    c_in = jnp.where(col >= L, col - L, col)
    mask = ((row >= L) == (col >= L)) & ((r_in < M) | (r_in >= c_in))
    NU = H // 2
    UW = 2 * E

    def qkv(hb, u):
        return tuple(
            jnp.dot(hb, _as_bf16(w[:, u * UW:(u + 1) * UW]), preferred_element_type=_F32)
            for w in (wq_v, wk_v, wv_v))

    def stack(t):
        return jnp.concatenate([t[:, :E], t[:, E:]], axis=0).astype(_BF16)

    def scores(q, k):
        sc = jax.lax.dot_general(stack(q), stack(k), (((1,), (1,)), ((), ())),
                                 preferred_element_type=_F32) * scale
        sc = jnp.where(mask, sc, -1e9)
        e = jnp.exp(sc - jnp.max(sc, axis=-1, keepdims=True))
        return (e / jnp.sum(e, axis=-1, keepdims=True)).astype(_BF16)

    def pv(p, v):
        o = jnp.dot(p, stack(v), preferred_element_type=_F32)
        return jnp.concatenate([o[:L], o[L:]], axis=1)

    def proj(o, u):
        return jnp.dot(o.astype(_BF16), _as_bf16(wo_v[u * E:(u + 1) * E, :]),
                       preferred_element_type=_F32)

    def half(hb, fix_qkv, fix_o):
        res = None
        saved = [None] * NU
        raw = qkv(hb, 0)
        prev_o = None
        for u in range(NU):
            q, k, v = fix_qkv(u, raw)
            p = scores(q, k)
            if u + 1 < NU:
                raw = qkv(hb, u + 1)
            elif prev_o is not None:
                d = proj(prev_o, u - 1)
                res = d if res is None else res + d
                prev_o = None
            o = pv(p, v)
            if prev_o is not None:
                d = proj(prev_o, u - 1)
                res = d if res is None else res + d
            prev_o, saved[u] = fix_o(u, o)
        d = proj(prev_o, NU - 1)
        return res + d, saved

    def pair_step(j, mem):
        r = pl.multiple_of(j * (2 * SEG), 2 * SEG)
        hb = jnp.concatenate([mem, xn_v[pl.ds(r, SEG + 8), :]], axis=0).astype(_BF16)
        extra = [None] * NU

        def fq_a(u, raw):
            extra[u] = tuple(t[L:] for t in raw)
            return tuple(t[:L] for t in raw)

        def fo_a(u, o):
            return o[:SEG], o[SEG:]

        res_a, tail_o = half(hb, fq_a, fo_a)
        mem = res_a[:M]
        hb = jnp.concatenate([mem, xn_v[pl.ds(r + SEG + 8, SEG - 8), :]], axis=0).astype(_BF16)

        def fq_b(u, raw):
            return tuple(jnp.concatenate([t[:M], ex, t[M:]], axis=0) for t, ex in zip(raw, extra[u]))

        def fo_b(u, o):
            return jnp.concatenate([o[:M], tail_o[u], o[M:]], axis=0), None

        res_b, _ = half(hb, fq_b, fo_b)
        s_all = jnp.concatenate([res_a[M:], res_b[M:]], axis=0)
        xr = x_v[pl.ds(r, 2 * SEG), :].astype(_F32)
        out_v[pl.ds(r, 2 * SEG), :] = (xr + s_all * gate_v[pl.ds(r, 2 * SEG), :]).astype(out_v.dtype)
        return res_b[:M]

    jax.lax.fori_loop(0, n_seg // 2, pair_step, mem0_ref[...].astype(_F32))

    cp_out = pltpu.make_async_copy(out_v, out_hbm, sems.at[0])
    cp_out.start()
    cp_out.wait()


@functools.partial(jax.jit, static_argnames=("A_seg_len",))
def pallas_recurrent_scan__memory_aug_recurrent_mem_tr__glu_gated_glu__prompt_kernel(
    A_x: jax.Array,
    A_mem0: jax.Array,
    A_Wq: jax.Array,
    A_Wk: jax.Array,
    A_Wv: jax.Array,
    A_Wo: jax.Array,
    A_seg_len: int,
    B_x: jax.Array,
    B_w_gate: jax.Array,
    B_w_up: jax.Array,
    B_w_down: jax.Array,
):
    del B_x
    B, S, D = A_x.shape
    _, H, E = A_Wq.shape
    M = A_mem0.shape[1]
    F = B_w_gate.shape[1]
    SEG = int(A_seg_len)
    assert B == 1 and S % SEG == 0

    kern = functools.partial(_kernel, S=S, D=D, H=H, E=E, M=M, SEG=SEG, F=F, MB=256, FC=512, HG=4)
    any_spec = pl.BlockSpec(memory_space=pl.ANY)
    out = pl.pallas_call(
        kern,
        out_shape=jax.ShapeDtypeStruct((S, D), A_x.dtype),
        in_specs=[any_spec, pl.BlockSpec(memory_space=pltpu.VMEM)] + [any_spec] * 7,
        out_specs=any_spec,
        scratch_shapes=[
            pltpu.VMEM((S, D), _BF16),
            pltpu.VMEM((S, D), _F32),
            pltpu.VMEM((S, D), _F32),
            pltpu.VMEM((S, D), _BF16),
            pltpu.VMEM((D // 2, H * E), _U32),
            pltpu.VMEM((D // 2, H * E), _U32),
            pltpu.VMEM((D // 2, H * E), _U32),
            pltpu.VMEM((H * E // 2, D), _U32),
            pltpu.VMEM((D // 2, F), _U32),
            pltpu.VMEM((D // 2, F), _U32),
            pltpu.VMEM((F // 2, D), _U32),
            pltpu.VMEM((2, 2, H // 2, D // 2, E), _U32),
            pltpu.SemaphoreType.DMA((8,)),
        ],
        compiler_params=pltpu.CompilerParams(vmem_limit_bytes=120 * 1024 * 1024),
    )(
        A_x.reshape(S, D),
        A_mem0.reshape(M, D),
        A_Wq.reshape(D // 2, 2, H, E),
        A_Wk.reshape(D // 2, 2, H, E),
        A_Wv.reshape(D // 2, 2, H, E),
        A_Wo.reshape(H * E, D),
        B_w_gate,
        B_w_up,
        B_w_down,
    )
    return out.reshape(B, S, D)
```

```python
import functools

import jax
import jax.numpy as jnp
import numpy as np
import jax.experimental.pallas as pl
import jax.experimental.pallas.tpu as pltpu

_F32 = jnp.float32
_BF16 = jnp.bfloat16
_U32 = jnp.uint32


def _as_bf16(w_u32):
    return pltpu.bitcast(w_u32, _BF16)


def _kernel(x_hbm, mem0_ref, wq_hbm, wk_hbm, wv_hbm, wo_hbm, wg_hbm, wu_hbm, wd_hbm,
            out_hbm,
            x_v, xn_v, gate_v, out_v, wq_v, wk_v, wv_v, wo_v, wg_v, wu_v, wd_v, st_v,
            sems,
            *, S, D, H, E, M, SEG, F, MB, FC, HG):
    n_seg = S // SEG
    scale = E ** (-0.5)
    L = M + SEG

    NC = F // FC
    NB = S // MB
    H2 = H // 2
    cp_x = pltpu.make_async_copy(x_hbm, x_v, sems.at[0])
    cp_o = pltpu.make_async_copy(wo_hbm.bitcast(_U32), wo_v, sems.at[1])

    def chunk_copies(c):
        return [
            pltpu.make_async_copy(wg_hbm.bitcast(_U32).at[:, pl.ds(c * FC, FC)],
                                  wg_v.at[:, pl.ds(c * FC, FC)], sems.at[4 + c]),
            pltpu.make_async_copy(wu_hbm.bitcast(_U32).at[:, pl.ds(c * FC, FC)],
                                  wu_v.at[:, pl.ds(c * FC, FC)], sems.at[4 + c]),
            pltpu.make_async_copy(wd_hbm.bitcast(_U32).at[pl.ds(c * (FC // 2), FC // 2), :],
                                  wd_v.at[pl.ds(c * (FC // 2), FC // 2), :], sems.at[4 + c]),
        ]

    def gather_copies(w_hbm, slot):
        wu = w_hbm.bitcast(_U32)
        return [pltpu.make_async_copy(wu.at[:, p, h2, :], st_v.at[slot, p, h2], sems.at[2 + slot])
                for p in range(2) for h2 in range(H2)]

    def start(cs):
        for c in cs:
            c.start()

    def wait(cs):
        for c in cs:
            c.wait()

    def repack(slot, dst, h2):
        a = st_v[slot, 0, h2]
        b = st_v[slot, 1, h2]
        lo = (a & 0xFFFF) | (b << 16)
        hi = (a >> 16) | (b & np.uint32(0xFFFF0000))
        c0 = pl.multiple_of(h2 * (2 * E), 2 * E)
        dst[:, pl.ds(c0, E)] = lo
        dst[:, pl.ds(c0 + E, E)] = hi

    def layernorm(i):
        r = pl.multiple_of(i * MB, MB)
        xv = x_v[pl.ds(r, MB), :].astype(_F32)
        mu = jnp.mean(xv, axis=-1, keepdims=True)
        xc = xv - mu
        var = jnp.mean(xc * xc, axis=-1, keepdims=True)
        xn_v[pl.ds(r, MB), :] = xc / jnp.sqrt(var + 1e-5)

    def glu_block(c, i):
        r = pl.multiple_of(i * MB, MB)
        xb = xn_v[pl.ds(r, MB), :].astype(_BF16)
        g = jnp.dot(xb, _as_bf16(wg_v[:, c * FC:(c + 1) * FC]), preferred_element_type=_F32)
        u = jnp.dot(xb, _as_bf16(wu_v[:, c * FC:(c + 1) * FC]), preferred_element_type=_F32)
        hh = (jax.nn.sigmoid(g) * u).astype(_BF16)
        d = jnp.dot(hh, _as_bf16(wd_v[c * (FC // 2):(c + 1) * (FC // 2), :]),
                    preferred_element_type=_F32)
        if c > 0:
            d = d + gate_v[pl.ds(r, MB), :]
        if c == NC - 1:
            d = jax.nn.silu(d)
        gate_v[pl.ds(r, MB), :] = d

    def glu_chunk(c, side=None):
        wait(chunk_copies(c))

        @pl.loop(0, NB)
        def _(i):
            glu_block(c, i)
            if side is not None:
                side(i)

    per = H2 // NB
    cp_x.start()
    start(chunk_copies(0))
    cp_x.wait()
    for c in range(1, NC):
        start(chunk_copies(c))
    cp_o.start()
    layernorm(0)
    glu_chunk(0, lambda i: layernorm(jnp.minimum(i + 1, NB - 1)))
    start(gather_copies(wq_hbm, 0))
    start(gather_copies(wk_hbm, 1))
    glu_chunk(1)
    wait(gather_copies(wq_hbm, 0))

    def side_repack(slot, dst):
        def f(i):
            for t in range(per):
                repack(slot, dst, i * per + t)
        return f

    glu_chunk(2, side_repack(0, wq_v))
    start(gather_copies(wv_hbm, 0))
    wait(gather_copies(wk_hbm, 1))
    glu_chunk(3, side_repack(1, wk_v))
    glu_chunk(4)
    wait(gather_copies(wv_hbm, 0))
    glu_chunk(5, side_repack(0, wv_v))
    for c in range(6, NC):
        glu_chunk(c)
    cp_o.wait()

    row = jax.lax.broadcasted_iota(jnp.int32, (2 * L, 2 * L), 0)
    col = jax.lax.broadcasted_iota(jnp.int32, (2 * L, 2 * L), 1)
    r_in = jnp.where(row >= L, row - L, row)
    c_in = jnp.where(col >= L, col - L, col)
    mask = ((row >= L) == (col >= L)) & ((r_in < M) | (r_in >= c_in))
    NU = H // 2
    UW = 2 * E

    def qkv(hb, u):
        return tuple(
            jnp.dot(hb, _as_bf16(w[:, u * UW:(u + 1) * UW]), preferred_element_type=_F32)
            for w in (wq_v, wk_v, wv_v))

    def stack(t):
        return jnp.concatenate([t[:, :E], t[:, E:]], axis=0).astype(_BF16)

    def scores(q, k):
        sc = jax.lax.dot_general(stack(q), stack(k), (((1,), (1,)), ((), ())),
                                 preferred_element_type=_F32) * scale
        sc = jnp.where(mask, sc, -1e9)
        e = jnp.exp(sc - jnp.max(sc, axis=-1, keepdims=True))
        return (e / jnp.sum(e, axis=-1, keepdims=True)).astype(_BF16)

    def pv(p, v):
        o = jnp.dot(p, stack(v), preferred_element_type=_F32)
        return jnp.concatenate([o[:L], o[L:]], axis=1)

    def proj(o, u):
        return jnp.dot(o.astype(_BF16), _as_bf16(wo_v[u * E:(u + 1) * E, :]),
                       preferred_element_type=_F32)

    def half(hb, fix_qkv, fix_o):
        res = None
        saved = [None] * NU
        raw = qkv(hb, 0)
        prev_o = None
        for u in range(NU):
            q, k, v = fix_qkv(u, raw)
            p = scores(q, k)
            if u + 1 < NU:
                raw = qkv(hb, u + 1)
            elif prev_o is not None:
                d = proj(prev_o, u - 1)
                res = d if res is None else res + d
                prev_o = None
            o = pv(p, v)
            if prev_o is not None:
                d = proj(prev_o, u - 1)
                res = d if res is None else res + d
            prev_o, saved[u] = fix_o(u, o)
        d = proj(prev_o, NU - 1)
        return res + d, saved

    def pair_step(j, mem):
        r = pl.multiple_of(j * (2 * SEG), 2 * SEG)
        hb = jnp.concatenate([mem, xn_v[pl.ds(r, SEG + 8), :]], axis=0).astype(_BF16)
        extra = [None] * NU

        def fq_a(u, raw):
            extra[u] = tuple(t[L:] for t in raw)
            return tuple(t[:L] for t in raw)

        def fo_a(u, o):
            return o[:SEG], o[SEG:]

        res_a, tail_o = half(hb, fq_a, fo_a)
        mem = res_a[:M]
        hb = jnp.concatenate([mem, xn_v[pl.ds(r + SEG + 8, SEG - 8), :]], axis=0).astype(_BF16)

        def fq_b(u, raw):
            return tuple(jnp.concatenate([t[:M], ex, t[M:]], axis=0) for t, ex in zip(raw, extra[u]))

        def fo_b(u, o):
            return jnp.concatenate([o[:M], tail_o[u], o[M:]], axis=0), None

        res_b, _ = half(hb, fq_b, fo_b)
        s_all = jnp.concatenate([res_a[M:], res_b[M:]], axis=0)
        xr = x_v[pl.ds(r, 2 * SEG), :].astype(_F32)
        out_v[pl.ds(r, 2 * SEG), :] = (xr + s_all * gate_v[pl.ds(r, 2 * SEG), :]).astype(out_v.dtype)
        pltpu.make_async_copy(out_v.at[pl.ds(r, 2 * SEG), :], out_hbm.at[pl.ds(r, 2 * SEG), :],
                              sems.at[0]).start()
        return res_b[:M]

    jax.lax.fori_loop(0, n_seg // 2, pair_step, mem0_ref[...].astype(_F32))

    pltpu.make_async_copy(out_v, out_hbm, sems.at[0]).wait()


@functools.partial(jax.jit, static_argnames=("A_seg_len",))
def pallas_recurrent_scan__memory_aug_recurrent_mem_tr__glu_gated_glu__prompt_kernel(
    A_x: jax.Array,
    A_mem0: jax.Array,
    A_Wq: jax.Array,
    A_Wk: jax.Array,
    A_Wv: jax.Array,
    A_Wo: jax.Array,
    A_seg_len: int,
    B_x: jax.Array,
    B_w_gate: jax.Array,
    B_w_up: jax.Array,
    B_w_down: jax.Array,
):
    del B_x
    B, S, D = A_x.shape
    _, H, E = A_Wq.shape
    M = A_mem0.shape[1]
    F = B_w_gate.shape[1]
    SEG = int(A_seg_len)
    assert B == 1 and S % SEG == 0

    kern = functools.partial(_kernel, S=S, D=D, H=H, E=E, M=M, SEG=SEG, F=F, MB=256, FC=512, HG=4)
    any_spec = pl.BlockSpec(memory_space=pl.ANY)
    out = pl.pallas_call(
        kern,
        out_shape=jax.ShapeDtypeStruct((S, D), A_x.dtype),
        in_specs=[any_spec, pl.BlockSpec(memory_space=pltpu.VMEM)] + [any_spec] * 7,
        out_specs=any_spec,
        scratch_shapes=[
            pltpu.VMEM((S, D), _BF16),
            pltpu.VMEM((S, D), _F32),
            pltpu.VMEM((S, D), _F32),
            pltpu.VMEM((S, D), _BF16),
            pltpu.VMEM((D // 2, H * E), _U32),
            pltpu.VMEM((D // 2, H * E), _U32),
            pltpu.VMEM((D // 2, H * E), _U32),
            pltpu.VMEM((H * E // 2, D), _U32),
            pltpu.VMEM((D // 2, F), _U32),
            pltpu.VMEM((D // 2, F), _U32),
            pltpu.VMEM((F // 2, D), _U32),
            pltpu.VMEM((2, 2, H // 2, D // 2, E), _U32),
            pltpu.SemaphoreType.DMA((4 + F // 512,)),
        ],
        compiler_params=pltpu.CompilerParams(vmem_limit_bytes=120 * 1024 * 1024),
    )(
        A_x.reshape(S, D),
        A_mem0.reshape(M, D),
        A_Wq.reshape(D // 2, 2, H, E),
        A_Wk.reshape(D // 2, 2, H, E),
        A_Wv.reshape(D // 2, 2, H, E),
        A_Wo.reshape(H * E, D),
        B_w_gate,
        B_w_up,
        B_w_down,
    )
    return out.reshape(B, S, D)
```

```python
import functools

import jax
import jax.numpy as jnp
import numpy as np
import jax.experimental.pallas as pl
import jax.experimental.pallas.tpu as pltpu

_F32 = jnp.float32
_BF16 = jnp.bfloat16
_U32 = jnp.uint32


def _as_bf16(w_u32):
    return pltpu.bitcast(w_u32, _BF16)


def _kernel(x_hbm, mem0_ref, wq_hbm, wk_hbm, wv_hbm, wo_hbm, wg_hbm, wu_hbm, wd_hbm,
            out_hbm,
            x_v, xn_v, gate_v, out_v, wq_v, wk_v, wv_v, wo_v, wg_v, wu_v, wd_v, st_v, s_v,
            sems,
            *, S, D, H, E, M, SEG, F, MB, FC, HG):
    n_seg = S // SEG
    scale = E ** (-0.5)
    L = M + SEG

    NC = F // FC
    NB = S // MB
    H2 = H // 2
    cp_x = pltpu.make_async_copy(x_hbm, x_v, sems.at[0])
    cp_o = pltpu.make_async_copy(wo_hbm.bitcast(_U32), wo_v, sems.at[1])

    def chunk_copies(c):
        return [
            pltpu.make_async_copy(wg_hbm.bitcast(_U32).at[:, pl.ds(c * FC, FC)],
                                  wg_v.at[:, pl.ds(c * FC, FC)], sems.at[4 + c]),
            pltpu.make_async_copy(wu_hbm.bitcast(_U32).at[:, pl.ds(c * FC, FC)],
                                  wu_v.at[:, pl.ds(c * FC, FC)], sems.at[4 + c]),
            pltpu.make_async_copy(wd_hbm.bitcast(_U32).at[pl.ds(c * (FC // 2), FC // 2), :],
                                  wd_v.at[pl.ds(c * (FC // 2), FC // 2), :], sems.at[4 + c]),
        ]

    def gather_copies(w_hbm, slot):
        wu = w_hbm.bitcast(_U32)
        return [pltpu.make_async_copy(wu.at[:, p, h2, :], st_v.at[slot, p, h2], sems.at[2 + slot])
                for p in range(2) for h2 in range(H2)]

    def start(cs):
        for c in cs:
            c.start()

    def wait(cs):
        for c in cs:
            c.wait()

    def repack(slot, dst, h2):
        a = st_v[slot, 0, h2]
        b = st_v[slot, 1, h2]
        lo = (a & 0xFFFF) | (b << 16)
        hi = (a >> 16) | (b & np.uint32(0xFFFF0000))
        c0 = pl.multiple_of(h2 * (2 * E), 2 * E)
        dst[:, pl.ds(c0, E)] = lo
        dst[:, pl.ds(c0 + E, E)] = hi

    def layernorm(i):
        r = pl.multiple_of(i * MB, MB)
        xv = x_v[pl.ds(r, MB), :].astype(_F32)
        mu = jnp.mean(xv, axis=-1, keepdims=True)
        xc = xv - mu
        var = jnp.mean(xc * xc, axis=-1, keepdims=True)
        xn_v[pl.ds(r, MB), :] = xc / jnp.sqrt(var + 1e-5)

    def glu_block(c, i):
        r = pl.multiple_of(i * MB, MB)
        xb = xn_v[pl.ds(r, MB), :].astype(_BF16)
        g = jnp.dot(xb, _as_bf16(wg_v[:, c * FC:(c + 1) * FC]), preferred_element_type=_F32)
        u = jnp.dot(xb, _as_bf16(wu_v[:, c * FC:(c + 1) * FC]), preferred_element_type=_F32)
        hh = (jax.nn.sigmoid(g) * u).astype(_BF16)
        d = jnp.dot(hh, _as_bf16(wd_v[c * (FC // 2):(c + 1) * (FC // 2), :]),
                    preferred_element_type=_F32)
        if c > 0:
            d = d + gate_v[pl.ds(r, MB), :]
        gate_v[pl.ds(r, MB), :] = d

    def glu_chunk(c, side=None):
        wait(chunk_copies(c))

        @pl.loop(0, NB)
        def _(i):
            glu_block(c, i)
            if side is not None:
                side(i)

    per = H2 // NB
    cp_x.start()
    start(chunk_copies(0))
    cp_x.wait()
    for c in range(1, NC):
        start(chunk_copies(c))
    cp_o.start()
    layernorm(0)
    glu_chunk(0, lambda i: layernorm(jnp.minimum(i + 1, NB - 1)))
    start(gather_copies(wq_hbm, 0))
    start(gather_copies(wk_hbm, 1))
    glu_chunk(1)
    wait(gather_copies(wq_hbm, 0))

    def side_repack(slot, dst):
        def f(i):
            for t in range(per):
                repack(slot, dst, i * per + t)
        return f

    glu_chunk(2, side_repack(0, wq_v))
    start(gather_copies(wv_hbm, 0))
    wait(gather_copies(wk_hbm, 1))
    glu_chunk(3, side_repack(1, wk_v))
    glu_chunk(4)
    wait(gather_copies(wv_hbm, 0))
    glu_chunk(5, side_repack(0, wv_v))
    for c in range(6, NC - 1):
        glu_chunk(c)
    wait(chunk_copies(NC - 1))
    cp_o.wait()
    s_v[...] = jnp.zeros_like(s_v)

    row = jax.lax.broadcasted_iota(jnp.int32, (2 * L, 2 * L), 0)
    col = jax.lax.broadcasted_iota(jnp.int32, (2 * L, 2 * L), 1)
    r_in = jnp.where(row >= L, row - L, row)
    c_in = jnp.where(col >= L, col - L, col)
    mask = ((row >= L) == (col >= L)) & ((r_in < M) | (r_in >= c_in))
    NU = H // 2
    UW = 2 * E

    def qkv(hb, u):
        return tuple(
            jnp.dot(hb, _as_bf16(w[:, u * UW:(u + 1) * UW]), preferred_element_type=_F32)
            for w in (wq_v, wk_v, wv_v))

    def stack(t):
        return jnp.concatenate([t[:, :E], t[:, E:]], axis=0).astype(_BF16)

    def scores(q, k):
        sc = jax.lax.dot_general(stack(q), stack(k), (((1,), (1,)), ((), ())),
                                 preferred_element_type=_F32) * scale
        sc = jnp.where(mask, sc, -1e9)
        e = jnp.exp(sc - jnp.max(sc, axis=-1, keepdims=True))
        return (e / jnp.sum(e, axis=-1, keepdims=True)).astype(_BF16)

    def pv(p, v):
        o = jnp.dot(p, stack(v), preferred_element_type=_F32)
        return jnp.concatenate([o[:L], o[L:]], axis=1)

    def proj(o, u):
        return jnp.dot(o.astype(_BF16), _as_bf16(wo_v[u * E:(u + 1) * E, :]),
                       preferred_element_type=_F32)

    def half(hb, fix_qkv, fix_o, fill):
        res = None
        saved = [None] * NU
        raw = qkv(hb, 0)
        prev_o = None
        for u in range(NU):
            q, k, v = fix_qkv(u, raw)
            p = scores(q, k)
            if u + 1 < NU:
                raw = qkv(hb, u + 1)
            elif prev_o is not None:
                d = proj(prev_o, u - 1)
                res = d if res is None else res + d
                prev_o = None
            o = pv(p, v)
            if prev_o is not None:
                d = proj(prev_o, u - 1)
                res = d if res is None else res + d
            prev_o, saved[u] = fix_o(u, o)
        filled = fill()
        d = proj(prev_o, NU - 1)
        return res + d, saved, filled

    def emit_out(r):
        xr = x_v[pl.ds(r, 2 * SEG), :].astype(_F32)
        gate = jax.nn.silu(gate_v[pl.ds(r, 2 * SEG), :])
        out_v[pl.ds(r, 2 * SEG), :] = (xr + s_v[...] * gate).astype(out_v.dtype)

    def out_copy(r):
        return pltpu.make_async_copy(out_v.at[pl.ds(r, 2 * SEG), :], out_hbm.at[pl.ds(r, 2 * SEG), :],
                                     sems.at[0])

    def pair_step(j, mem):
        r = pl.multiple_of(j * (2 * SEG), 2 * SEG)
        hb = jnp.concatenate([mem, xn_v[pl.ds(r, SEG + 8), :]], axis=0).astype(_BF16)
        extra = [None] * NU

        def fq_a(u, raw):
            extra[u] = tuple(t[L:] for t in raw)
            return tuple(t[:L] for t in raw)

        def fo_a(u, o):
            return o[:SEG], o[SEG:]

        c = NC - 1
        xb = xn_v[pl.ds(r, 2 * SEG), :].astype(_BF16)

        def fill_a():
            return jnp.dot(xb, _as_bf16(wg_v[:, c * FC:(c + 1) * FC]), preferred_element_type=_F32)

        res_a, tail_o, g = half(hb, fq_a, fo_a, fill_a)
        u_ = jnp.dot(xb, _as_bf16(wu_v[:, c * FC:(c + 1) * FC]), preferred_element_type=_F32)
        hh = (jax.nn.sigmoid(g) * u_).astype(_BF16)
        mem = res_a[:M]
        rp = pl.multiple_of(jnp.maximum(j - 1, 0) * (2 * SEG), 2 * SEG)
        emit_out(rp)
        hb = jnp.concatenate([mem, xn_v[pl.ds(r + SEG + 8, SEG - 8), :]], axis=0).astype(_BF16)

        def fq_b(u, raw):
            return tuple(jnp.concatenate([t[:M], ex, t[M:]], axis=0) for t, ex in zip(raw, extra[u]))

        def fo_b(u, o):
            return jnp.concatenate([o[:M], tail_o[u], o[M:]], axis=0), None

        def fill_b():
            return jnp.dot(hh, _as_bf16(wd_v[c * (FC // 2):(c + 1) * (FC // 2), :]),
                           preferred_element_type=_F32)

        res_b, _, d = half(hb, fq_b, fo_b, fill_b)
        gate_v[pl.ds(r, 2 * SEG), :] += d
        s_v[:SEG - 8, :] = res_a[M:]
        s_v[SEG - 8:, :] = res_b[M:]

        @pl.when(j > 0)
        def _():
            out_copy(rp).start()

        return res_b[:M]

    jax.lax.fori_loop(0, n_seg // 2, pair_step, mem0_ref[...].astype(_F32))
    r_last = S - 2 * SEG
    emit_out(r_last)
    out_copy(r_last).start()

    pltpu.make_async_copy(out_v, out_hbm, sems.at[0]).wait()


@functools.partial(jax.jit, static_argnames=("A_seg_len",))
def pallas_recurrent_scan__memory_aug_recurrent_mem_tr__glu_gated_glu__prompt_kernel(
    A_x: jax.Array,
    A_mem0: jax.Array,
    A_Wq: jax.Array,
    A_Wk: jax.Array,
    A_Wv: jax.Array,
    A_Wo: jax.Array,
    A_seg_len: int,
    B_x: jax.Array,
    B_w_gate: jax.Array,
    B_w_up: jax.Array,
    B_w_down: jax.Array,
):
    del B_x
    B, S, D = A_x.shape
    _, H, E = A_Wq.shape
    M = A_mem0.shape[1]
    F = B_w_gate.shape[1]
    SEG = int(A_seg_len)
    assert B == 1 and S % SEG == 0

    kern = functools.partial(_kernel, S=S, D=D, H=H, E=E, M=M, SEG=SEG, F=F, MB=256, FC=512, HG=4)
    any_spec = pl.BlockSpec(memory_space=pl.ANY)
    out = pl.pallas_call(
        kern,
        out_shape=jax.ShapeDtypeStruct((S, D), A_x.dtype),
        in_specs=[any_spec, pl.BlockSpec(memory_space=pltpu.VMEM)] + [any_spec] * 7,
        out_specs=any_spec,
        scratch_shapes=[
            pltpu.VMEM((S, D), _BF16),
            pltpu.VMEM((S, D), _F32),
            pltpu.VMEM((S, D), _F32),
            pltpu.VMEM((S, D), _BF16),
            pltpu.VMEM((D // 2, H * E), _U32),
            pltpu.VMEM((D // 2, H * E), _U32),
            pltpu.VMEM((D // 2, H * E), _U32),
            pltpu.VMEM((H * E // 2, D), _U32),
            pltpu.VMEM((D // 2, F), _U32),
            pltpu.VMEM((D // 2, F), _U32),
            pltpu.VMEM((F // 2, D), _U32),
            pltpu.VMEM((2, 2, H // 2, D // 2, E), _U32),
            pltpu.VMEM((2 * SEG, D), _F32),
            pltpu.SemaphoreType.DMA((4 + F // 512,)),
        ],
        compiler_params=pltpu.CompilerParams(vmem_limit_bytes=120 * 1024 * 1024),
    )(
        A_x.reshape(S, D),
        A_mem0.reshape(M, D),
        A_Wq.reshape(D // 2, 2, H, E),
        A_Wk.reshape(D // 2, 2, H, E),
        A_Wv.reshape(D // 2, 2, H, E),
        A_Wo.reshape(H * E, D),
        B_w_gate,
        B_w_up,
        B_w_down,
    )
    return out.reshape(B, S, D)
```

```python
import functools

import jax
import jax.numpy as jnp
import numpy as np
import jax.experimental.pallas as pl
import jax.experimental.pallas.tpu as pltpu

_F32 = jnp.float32
_BF16 = jnp.bfloat16
_U32 = jnp.uint32


def _as_bf16(w_u32):
    return pltpu.bitcast(w_u32, _BF16)


def _kernel(x_hbm, mem0_ref, wq_hbm, wk_hbm, wv_hbm, wo_hbm, wg_hbm, wu_hbm, wd_hbm,
            out_hbm,
            x_v, xn_v, gate_v, out_v, wq_v, wk_v, wv_v, wo_v, wg_v, wu_v, wd_v, st_v, s_v, sg_v, sd_v,
            sems,
            *, S, D, H, E, M, SEG, F, MB, FC, HG):
    n_seg = S // SEG
    scale = E ** (-0.5)
    L = M + SEG

    NC = F // FC
    NB = S // MB
    H2 = H // 2
    cp_x = pltpu.make_async_copy(x_hbm, x_v, sems.at[0])
    cp_o = pltpu.make_async_copy(wo_hbm.bitcast(_U32), wo_v, sems.at[1])

    def chunk_copies(c):
        return [
            pltpu.make_async_copy(wg_hbm.bitcast(_U32).at[:, pl.ds(c * FC, FC)],
                                  wg_v.at[:, pl.ds(c * FC, FC)], sems.at[4 + c]),
            pltpu.make_async_copy(wu_hbm.bitcast(_U32).at[:, pl.ds(c * FC, FC)],
                                  wu_v.at[:, pl.ds(c * FC, FC)], sems.at[4 + c]),
            pltpu.make_async_copy(wd_hbm.bitcast(_U32).at[pl.ds(c * (FC // 2), FC // 2), :],
                                  wd_v.at[pl.ds(c * (FC // 2), FC // 2), :], sems.at[4 + c]),
        ]

    def gather_copies(w_hbm, slot):
        wu = w_hbm.bitcast(_U32)
        return [pltpu.make_async_copy(wu.at[:, p, h2, :], st_v.at[slot, p, h2], sems.at[2 + slot])
                for p in range(2) for h2 in range(H2)]

    def start(cs):
        for c in cs:
            c.start()

    def wait(cs):
        for c in cs:
            c.wait()

    def repack(slot, dst, h2):
        a = st_v[slot, 0, h2]
        b = st_v[slot, 1, h2]
        lo = (a & 0xFFFF) | (b << 16)
        hi = (a >> 16) | (b & np.uint32(0xFFFF0000))
        c0 = pl.multiple_of(h2 * (2 * E), 2 * E)
        dst[:, pl.ds(c0, E)] = lo
        dst[:, pl.ds(c0 + E, E)] = hi

    def layernorm(i):
        r = pl.multiple_of(i * MB, MB)
        xv = x_v[pl.ds(r, MB), :].astype(_F32)
        mu = jnp.mean(xv, axis=-1, keepdims=True)
        xc = xv - mu
        var = jnp.mean(xc * xc, axis=-1, keepdims=True)
        xn_v[pl.ds(r, MB), :] = xc / jnp.sqrt(var + 1e-5)

    def glu_block(c, i):
        r = pl.multiple_of(i * MB, MB)
        xb = xn_v[pl.ds(r, MB), :].astype(_BF16)
        g = jnp.dot(xb, _as_bf16(wg_v[:, c * FC:(c + 1) * FC]), preferred_element_type=_F32)
        u = jnp.dot(xb, _as_bf16(wu_v[:, c * FC:(c + 1) * FC]), preferred_element_type=_F32)
        hh = (jax.nn.sigmoid(g) * u).astype(_BF16)
        d = jnp.dot(hh, _as_bf16(wd_v[c * (FC // 2):(c + 1) * (FC // 2), :]),
                    preferred_element_type=_F32)
        if c > 0:
            d = d + gate_v[pl.ds(r, MB), :]
        gate_v[pl.ds(r, MB), :] = d

    KH, FH, DH, MH = D // 4, FC // 4, D // 2, MB // 2

    def w_blocks(c, lo, n, lo2, n2):
        return ((wg_v[pl.ds(lo, n), c * FC:(c + 1) * FC], wu_v[pl.ds(lo, n), c * FC:(c + 1) * FC],
                 wg_v[pl.ds(KH + lo, n), c * FC:(c + 1) * FC], wu_v[pl.ds(KH + lo, n), c * FC:(c + 1) * FC]),
                (wd_v[pl.ds(2 * c * FH + lo2, n2), :DH], wd_v[pl.ds(2 * c * FH + lo2, n2), DH:],
                 wd_v[pl.ds((2 * c + 1) * FH + lo2, n2), :DH], wd_v[pl.ds((2 * c + 1) * FH + lo2, n2), DH:]))

    def w_sums(b):
        w11, w12, w21, w22 = (_as_bf16(t).astype(_F32) for t in b)
        return [pltpu.bitcast(t.astype(_BF16), _U32)
                for t in (w11 + w22, w12 - w22, w21 - w11, w11 + w12, w21 + w22)]

    def prep(c, i):
        n, n2 = KH // NB, FH // NB
        lo, lo2 = pl.multiple_of(i * n, n), pl.multiple_of(i * n2, n2)
        gu, dn = w_blocks(c, lo, n, lo2, n2)
        for t, v in enumerate(w_sums(gu)):
            sg_v[c % 2, t, pl.ds(lo, n), :] = v
        for t, v in enumerate(w_sums(dn)):
            sd_v[c % 2, t, pl.ds(lo2, n2), :] = v

    def strassen(a, hr, hc, w11, w22, sums):
        a11, a12, a21, a22 = a[:hr, :hc], a[:hr, hc:], a[hr:, :hc], a[hr:, hc:]
        mm = lambda l, w: jnp.dot(l.astype(_BF16), _as_bf16(w), preferred_element_type=_F32)
        m1 = mm(a11 + a22, sums(0))
        m2 = mm(a21 + a22, w11)
        m3 = mm(a11, sums(1))
        m4 = mm(a22, sums(2))
        m5 = mm(a11 + a12, w22)
        m6 = mm(a21 - a11, sums(3))
        m7 = mm(a12 - a22, sums(4))
        return m1 + m4 - m5 + m7, m3 + m5, m2 + m4, m1 - m2 + m3 + m6

    def glu_block_s(c, i):
        r = pl.multiple_of(i * MB, MB)
        (g11, _, _, u22), (d11, _, _, d22) = w_blocks(c, 0, KH, 0, FH)
        c11, c12, c21, c22 = strassen(xn_v[pl.ds(r, MB), :], MH, D // 2, g11, u22,
                                      lambda t: sg_v[c % 2, t])
        hh = jnp.concatenate([jax.nn.sigmoid(c11) * c12, jax.nn.sigmoid(c21) * c22], axis=0)
        o11, o12, o21, o22 = strassen(hh, MH, FC // 2, d11, d22, lambda t: sd_v[c % 2, t])
        r2 = pl.multiple_of(r + MH, MH)
        gate_v[pl.ds(r, MH), :DH] += o11
        gate_v[pl.ds(r, MH), DH:] += o12
        gate_v[pl.ds(r2, MH), :DH] += o21
        gate_v[pl.ds(r2, MH), DH:] += o22

    def glu_chunk(c, side=None):
        if c == 0:
            wait(chunk_copies(c))
        else:
            if c == 1:
                wait(chunk_copies(1))
                pl.loop(0, NB)(lambda i: prep(1, i))
            if c + 1 < NC - 1:
                wait(chunk_copies(c + 1))

        @pl.loop(0, NB)
        def _(i):
            if c == 0:
                glu_block(c, i)
            else:
                glu_block_s(c, i)
                if c + 1 < NC - 1:
                    prep(c + 1, i)
            if side is not None:
                side(i)

    per = H2 // NB
    cp_x.start()
    start(chunk_copies(0))
    cp_x.wait()
    for c in range(1, NC):
        start(chunk_copies(c))
    cp_o.start()
    layernorm(0)
    glu_chunk(0, lambda i: layernorm(jnp.minimum(i + 1, NB - 1)))
    start(gather_copies(wq_hbm, 0))
    start(gather_copies(wk_hbm, 1))
    glu_chunk(1)
    wait(gather_copies(wq_hbm, 0))

    def side_repack(slot, dst):
        def f(i):
            for t in range(per):
                repack(slot, dst, i * per + t)
        return f

    glu_chunk(2, side_repack(0, wq_v))
    start(gather_copies(wv_hbm, 0))
    wait(gather_copies(wk_hbm, 1))
    glu_chunk(3, side_repack(1, wk_v))
    glu_chunk(4)
    wait(gather_copies(wv_hbm, 0))
    glu_chunk(5, side_repack(0, wv_v))
    for c in range(6, NC - 1):
        glu_chunk(c)
    wait(chunk_copies(NC - 1))
    cp_o.wait()
    s_v[...] = jnp.zeros_like(s_v)

    row = jax.lax.broadcasted_iota(jnp.int32, (2 * L, 2 * L), 0)
    col = jax.lax.broadcasted_iota(jnp.int32, (2 * L, 2 * L), 1)
    r_in = jnp.where(row >= L, row - L, row)
    c_in = jnp.where(col >= L, col - L, col)
    mask = ((row >= L) == (col >= L)) & ((r_in < M) | (r_in >= c_in))
    NU = H // 2
    UW = 2 * E

    def qkv(hb, u):
        return tuple(
            jnp.dot(hb, _as_bf16(w[:, u * UW:(u + 1) * UW]), preferred_element_type=_F32)
            for w in (wq_v, wk_v, wv_v))

    def stack(t):
        return jnp.concatenate([t[:, :E], t[:, E:]], axis=0).astype(_BF16)

    def scores(q, k):
        sc = jax.lax.dot_general(stack(q), stack(k), (((1,), (1,)), ((), ())),
                                 preferred_element_type=_F32) * scale
        sc = jnp.where(mask, sc, -1e9)
        e = jnp.exp(sc - jnp.max(sc, axis=-1, keepdims=True))
        return (e / jnp.sum(e, axis=-1, keepdims=True)).astype(_BF16)

    def pv(p, v):
        o = jnp.dot(p, stack(v), preferred_element_type=_F32)
        return jnp.concatenate([o[:L], o[L:]], axis=1)

    def proj(o, u):
        return jnp.dot(o.astype(_BF16), _as_bf16(wo_v[u * E:(u + 1) * E, :]),
                       preferred_element_type=_F32)

    def half(hb, fix_qkv, fix_o, fill):
        res = None
        saved = [None] * NU
        raw = qkv(hb, 0)
        prev_o = None
        for u in range(NU):
            q, k, v = fix_qkv(u, raw)
            p = scores(q, k)
            if u + 1 < NU:
                raw = qkv(hb, u + 1)
            elif prev_o is not None:
                d = proj(prev_o, u - 1)
                res = d if res is None else res + d
                prev_o = None
            o = pv(p, v)
            if prev_o is not None:
                d = proj(prev_o, u - 1)
                res = d if res is None else res + d
            prev_o, saved[u] = fix_o(u, o)
        filled = fill()
        d = proj(prev_o, NU - 1)
        return res + d, saved, filled

    def emit_out(r):
        xr = x_v[pl.ds(r, 2 * SEG), :].astype(_F32)
        gate = jax.nn.silu(gate_v[pl.ds(r, 2 * SEG), :])
        out_v[pl.ds(r, 2 * SEG), :] = (xr + s_v[...] * gate).astype(out_v.dtype)

    def out_copy(r):
        return pltpu.make_async_copy(out_v.at[pl.ds(r, 2 * SEG), :], out_hbm.at[pl.ds(r, 2 * SEG), :],
                                     sems.at[0])

    def pair_step(j, mem):
        r = pl.multiple_of(j * (2 * SEG), 2 * SEG)
        hb = jnp.concatenate([mem, xn_v[pl.ds(r, SEG + 8), :]], axis=0).astype(_BF16)
        extra = [None] * NU

        def fq_a(u, raw):
            extra[u] = tuple(t[L:] for t in raw)
            return tuple(t[:L] for t in raw)

        def fo_a(u, o):
            return o[:SEG], o[SEG:]

        c = NC - 1
        xb = xn_v[pl.ds(r, 2 * SEG), :].astype(_BF16)

        def fill_a():
            return jnp.dot(xb, _as_bf16(wg_v[:, c * FC:(c + 1) * FC]), preferred_element_type=_F32)

        res_a, tail_o, g = half(hb, fq_a, fo_a, fill_a)
        u_ = jnp.dot(xb, _as_bf16(wu_v[:, c * FC:(c + 1) * FC]), preferred_element_type=_F32)
        hh = (jax.nn.sigmoid(g) * u_).astype(_BF16)
        mem = res_a[:M]
        rp = pl.multiple_of(jnp.maximum(j - 1, 0) * (2 * SEG), 2 * SEG)
        emit_out(rp)
        hb = jnp.concatenate([mem, xn_v[pl.ds(r + SEG + 8, SEG - 8), :]], axis=0).astype(_BF16)

        def fq_b(u, raw):
            return tuple(jnp.concatenate([t[:M], ex, t[M:]], axis=0) for t, ex in zip(raw, extra[u]))

        def fo_b(u, o):
            return jnp.concatenate([o[:M], tail_o[u], o[M:]], axis=0), None

        def fill_b():
            return jnp.dot(hh, _as_bf16(wd_v[c * (FC // 2):(c + 1) * (FC // 2), :]),
                           preferred_element_type=_F32)

        res_b, _, d = half(hb, fq_b, fo_b, fill_b)
        gate_v[pl.ds(r, 2 * SEG), :] += d
        s_v[:SEG - 8, :] = res_a[M:]
        s_v[SEG - 8:, :] = res_b[M:]

        @pl.when(j > 0)
        def _():
            out_copy(rp).start()

        return res_b[:M]

    jax.lax.fori_loop(0, n_seg // 2, pair_step, mem0_ref[...].astype(_F32))
    r_last = S - 2 * SEG
    emit_out(r_last)
    out_copy(r_last).start()

    pltpu.make_async_copy(out_v, out_hbm, sems.at[0]).wait()


@functools.partial(jax.jit, static_argnames=("A_seg_len",))
def pallas_recurrent_scan__memory_aug_recurrent_mem_tr__glu_gated_glu__prompt_kernel(
    A_x: jax.Array,
    A_mem0: jax.Array,
    A_Wq: jax.Array,
    A_Wk: jax.Array,
    A_Wv: jax.Array,
    A_Wo: jax.Array,
    A_seg_len: int,
    B_x: jax.Array,
    B_w_gate: jax.Array,
    B_w_up: jax.Array,
    B_w_down: jax.Array,
):
    del B_x
    B, S, D = A_x.shape
    _, H, E = A_Wq.shape
    M = A_mem0.shape[1]
    F = B_w_gate.shape[1]
    SEG = int(A_seg_len)
    assert B == 1 and S % SEG == 0

    kern = functools.partial(_kernel, S=S, D=D, H=H, E=E, M=M, SEG=SEG, F=F, MB=256, FC=512, HG=4)
    any_spec = pl.BlockSpec(memory_space=pl.ANY)
    out = pl.pallas_call(
        kern,
        out_shape=jax.ShapeDtypeStruct((S, D), A_x.dtype),
        in_specs=[any_spec, pl.BlockSpec(memory_space=pltpu.VMEM)] + [any_spec] * 7,
        out_specs=any_spec,
        scratch_shapes=[
            pltpu.VMEM((S, D), _BF16),
            pltpu.VMEM((S, D), _F32),
            pltpu.VMEM((S, D), _F32),
            pltpu.VMEM((S, D), _BF16),
            pltpu.VMEM((D // 2, H * E), _U32),
            pltpu.VMEM((D // 2, H * E), _U32),
            pltpu.VMEM((D // 2, H * E), _U32),
            pltpu.VMEM((H * E // 2, D), _U32),
            pltpu.VMEM((D // 2, F), _U32),
            pltpu.VMEM((D // 2, F), _U32),
            pltpu.VMEM((F // 2, D), _U32),
            pltpu.VMEM((2, 2, H // 2, D // 2, E), _U32),
            pltpu.VMEM((2 * SEG, D), _F32),
            pltpu.VMEM((2, 5, D // 4, 512), _U32),
            pltpu.VMEM((2, 5, 128, D // 2), _U32),
            pltpu.SemaphoreType.DMA((4 + F // 512,)),
        ],
        compiler_params=pltpu.CompilerParams(vmem_limit_bytes=120 * 1024 * 1024),
    )(
        A_x.reshape(S, D),
        A_mem0.reshape(M, D),
        A_Wq.reshape(D // 2, 2, H, E),
        A_Wk.reshape(D // 2, 2, H, E),
        A_Wv.reshape(D // 2, 2, H, E),
        A_Wo.reshape(H * E, D),
        B_w_gate,
        B_w_up,
        B_w_down,
    )
    return out.reshape(B, S, D)
```

```python
import functools

import jax
import jax.numpy as jnp
import numpy as np
import jax.experimental.pallas as pl
import jax.experimental.pallas.tpu as pltpu

_F32 = jnp.float32
_BF16 = jnp.bfloat16
_U32 = jnp.uint32


def _as_bf16(w_u32):
    return pltpu.bitcast(w_u32, _BF16)


def _kernel(x_hbm, mem0_ref, wq_hbm, wk_hbm, wv_hbm, wo_hbm, wg_hbm, wu_hbm, wd_hbm,
            out_hbm,
            x_v, xn_v, gate_v, out_v, wq_v, wk_v, wv_v, wo_v, wg_v, wu_v, wd_v, st_v, s_v, sg_v, sd_v,
            sems,
            *, S, D, H, E, M, SEG, F, MB, FC, HG):
    n_seg = S // SEG
    scale = E ** (-0.5)
    L = M + SEG

    NC = F // FC
    NB = S // MB
    H2 = H // 2
    cp_x0 = pltpu.make_async_copy(x_hbm.at[pl.ds(0, MB)], x_v.at[pl.ds(0, MB)], sems.at[0])
    cp_x = pltpu.make_async_copy(x_hbm.at[pl.ds(MB, S - MB)], x_v.at[pl.ds(MB, S - MB)], sems.at[2])
    cp_o = pltpu.make_async_copy(wo_hbm.bitcast(_U32), wo_v, sems.at[1])

    def chunk_copies(c):
        return [
            pltpu.make_async_copy(wg_hbm.bitcast(_U32).at[:, pl.ds(c * FC, FC)],
                                  wg_v.at[:, pl.ds(c * FC, FC)], sems.at[4 + c]),
            pltpu.make_async_copy(wu_hbm.bitcast(_U32).at[:, pl.ds(c * FC, FC)],
                                  wu_v.at[:, pl.ds(c * FC, FC)], sems.at[4 + c]),
            pltpu.make_async_copy(wd_hbm.bitcast(_U32).at[pl.ds(c * (FC // 2), FC // 2), :],
                                  wd_v.at[pl.ds(c * (FC // 2), FC // 2), :], sems.at[4 + c]),
        ]

    def gather_copies(w_hbm, slot):
        wu = w_hbm.bitcast(_U32)
        return [pltpu.make_async_copy(wu.at[:, p, h2, :], st_v.at[slot, p, h2], sems.at[2 + slot])
                for p in range(2) for h2 in range(H2)]

    def start(cs):
        for c in cs:
            c.start()

    def wait(cs):
        for c in cs:
            c.wait()

    def repack(slot, dst, h2):
        a = st_v[slot, 0, h2]
        b = st_v[slot, 1, h2]
        lo = (a & 0xFFFF) | (b << 16)
        hi = (a >> 16) | (b & np.uint32(0xFFFF0000))
        c0 = pl.multiple_of(h2 * (2 * E), 2 * E)
        dst[:, pl.ds(c0, E)] = lo
        dst[:, pl.ds(c0 + E, E)] = hi

    def layernorm(i):
        r = pl.multiple_of(i * MB, MB)
        xv = x_v[pl.ds(r, MB), :].astype(_F32)
        mu = jnp.mean(xv, axis=-1, keepdims=True)
        xc = xv - mu
        var = jnp.mean(xc * xc, axis=-1, keepdims=True)
        xn_v[pl.ds(r, MB), :] = xc / jnp.sqrt(var + 1e-5)

    KH, FH, DH, MH = D // 4, FC // 4, D // 2, MB // 2

    def w_blocks(c, lo, n, lo2, n2):
        return ((wg_v[pl.ds(lo, n), c * FC:(c + 1) * FC], wu_v[pl.ds(lo, n), c * FC:(c + 1) * FC],
                 wg_v[pl.ds(KH + lo, n), c * FC:(c + 1) * FC], wu_v[pl.ds(KH + lo, n), c * FC:(c + 1) * FC]),
                (wd_v[pl.ds(2 * c * FH + lo2, n2), :DH], wd_v[pl.ds(2 * c * FH + lo2, n2), DH:],
                 wd_v[pl.ds((2 * c + 1) * FH + lo2, n2), :DH], wd_v[pl.ds((2 * c + 1) * FH + lo2, n2), DH:]))

    def w_sums(b):
        w11, w12, w21, w22 = (_as_bf16(t).astype(_F32) for t in b)
        return [pltpu.bitcast(t.astype(_BF16), _U32)
                for t in (w11 + w22, w12 - w22, w21 - w11, w11 + w12, w21 + w22)]

    def prep(c, i):
        n, n2 = KH // NB, FH // NB
        lo, lo2 = pl.multiple_of(i * n, n), pl.multiple_of(i * n2, n2)
        gu, dn = w_blocks(c, lo, n, lo2, n2)
        for t, v in enumerate(w_sums(gu)):
            sg_v[c % 2, t, pl.ds(lo, n), :] = v
        for t, v in enumerate(w_sums(dn)):
            sd_v[c % 2, t, pl.ds(lo2, n2), :] = v

    def mm(l, w):
        return jnp.dot(l.astype(_BF16), _as_bf16(w), preferred_element_type=_F32)

    def acc(c, rows, cols, v):
        if c == 0:
            gate_v[rows, cols] = v
        else:
            gate_v[rows, cols] += v

    def glu_block_s(c, i):
        r = pl.multiple_of(i * MB, MB)
        r2 = pl.multiple_of(r + MH, MH)
        (w11, _, _, w22), (d11, _, _, d22) = w_blocks(c, 0, KH, 0, FH)
        sg = lambda t: sg_v[c % 2, t]
        sd = lambda t: sd_v[c % 2, t]
        a11, a12 = xn_v[pl.ds(r, MH), :DH], xn_v[pl.ds(r, MH), DH:]
        a21, a22 = xn_v[pl.ds(r2, MH), :DH], xn_v[pl.ds(r2, MH), DH:]
        m4 = mm(a22, sg(2))
        m1 = mm(a11 + a22, sg(0))
        m5 = mm(a11 + a12, w22)
        m7 = mm(a12 - a22, sg(4))
        g_top = m1 + m4 - m5 + m7
        m3 = mm(a11, sg(1))
        h_top = jax.nn.sigmoid(g_top) * (m3 + m5)
        m2 = mm(a21 + a22, w11)
        m6 = mm(a21 - a11, sg(3))
        h_bot = jax.nn.sigmoid(m2 + m4) * (m1 - m2 + m3 + m6)
        FQ = FC // 2
        b11, b12, b21, b22 = h_top[:, :FQ], h_top[:, FQ:], h_bot[:, :FQ], h_bot[:, FQ:]
        n3 = mm(b11, sd(1))
        n5 = mm(b11 + b12, d22)
        acc(c, pl.ds(r, MH), slice(DH, D), n3 + n5)
        n1 = mm(b11 + b22, sd(0))
        n4 = mm(b22, sd(2))
        n7 = mm(b12 - b22, sd(4))
        acc(c, pl.ds(r, MH), slice(0, DH), n1 + n4 - n5 + n7)
        n2 = mm(b21 + b22, d11)
        acc(c, pl.ds(r2, MH), slice(0, DH), n2 + n4)
        n6 = mm(b21 - b11, sd(3))
        acc(c, pl.ds(r2, MH), slice(DH, D), n1 - n2 + n3 + n6)

    def glu_chunk(c, side=None, lo=0, hi=None, do_prep=True):
        @pl.loop(lo, NB if hi is None else hi)
        def _(i):
            glu_block_s(c, i)
            if do_prep and c + 1 < NC - 1:
                prep(c + 1, i)
            if side is not None:
                side(i)

    per = H2 // NB
    cp_x0.start()
    start(chunk_copies(0))
    cp_x.start()
    cp_x0.wait()
    layernorm(0)
    wait(chunk_copies(0))
    for c in range(1, NC):
        start(chunk_copies(c))
    cp_o.start()
    pl.loop(0, NB)(lambda i: prep(0, i))
    cp_x.wait()
    ln_next = lambda i: layernorm(jnp.minimum(i + 1, NB - 1))
    glu_chunk(0, ln_next, hi=NB // 2, do_prep=False)
    wait(chunk_copies(1))

    def side0(i):
        ln_next(i)
        prep(1, 2 * i - NB)
        prep(1, 2 * i - NB + 1)

    glu_chunk(0, side0, lo=NB // 2, do_prep=False)
    for c in range(2, NC - 1):
        wait(chunk_copies(c))
    start(gather_copies(wq_hbm, 0))
    start(gather_copies(wk_hbm, 1))
    glu_chunk(1)
    wait(gather_copies(wq_hbm, 0))

    def side_repack(slot, dst):
        def f(i):
            for t in range(per):
                repack(slot, dst, i * per + t)
        return f

    glu_chunk(2, side_repack(0, wq_v))
    start(gather_copies(wv_hbm, 0))
    wait(gather_copies(wk_hbm, 1))
    glu_chunk(3, side_repack(1, wk_v))
    glu_chunk(4)
    wait(gather_copies(wv_hbm, 0))
    glu_chunk(5, side_repack(0, wv_v))
    for c in range(6, NC - 1):
        glu_chunk(c)
    wait(chunk_copies(NC - 1))
    cp_o.wait()
    s_v[...] = jnp.zeros_like(s_v)

    row = jax.lax.broadcasted_iota(jnp.int32, (2 * L, 2 * L), 0)
    col = jax.lax.broadcasted_iota(jnp.int32, (2 * L, 2 * L), 1)
    r_in = jnp.where(row >= L, row - L, row)
    c_in = jnp.where(col >= L, col - L, col)
    mask = ((row >= L) == (col >= L)) & ((r_in < M) | (r_in >= c_in))
    NU = H // 2
    UW = 2 * E

    def qkv(hb, u):
        return tuple(
            jnp.dot(hb, _as_bf16(w[:, u * UW:(u + 1) * UW]), preferred_element_type=_F32)
            for w in (wq_v, wk_v, wv_v))

    def stack(t):
        return jnp.concatenate([t[:, :E], t[:, E:]], axis=0).astype(_BF16)

    def scores(q, k):
        sc = jax.lax.dot_general(stack(q), stack(k), (((1,), (1,)), ((), ())),
                                 preferred_element_type=_F32) * scale
        sc = jnp.where(mask, sc, -1e9)
        e = jnp.exp(sc - jnp.max(sc, axis=-1, keepdims=True))
        return (e / jnp.sum(e, axis=-1, keepdims=True)).astype(_BF16)

    def pv(p, v):
        o = jnp.dot(p, stack(v), preferred_element_type=_F32)
        return jnp.concatenate([o[:L], o[L:]], axis=1)

    def proj(o, u):
        return jnp.dot(o.astype(_BF16), _as_bf16(wo_v[u * E:(u + 1) * E, :]),
                       preferred_element_type=_F32)

    def half(hb, fix_qkv, fix_o, fill):
        res = None
        saved = [None] * NU
        raw = qkv(hb, 0)
        prev_o = None
        for u in range(NU):
            q, k, v = fix_qkv(u, raw)
            p = scores(q, k)
            if u + 1 < NU:
                raw = qkv(hb, u + 1)
            elif prev_o is not None:
                d = proj(prev_o, u - 1)
                res = d if res is None else res + d
                prev_o = None
            o = pv(p, v)
            if prev_o is not None:
                d = proj(prev_o, u - 1)
                res = d if res is None else res + d
            prev_o, saved[u] = fix_o(u, o)
        filled = fill()
        d = proj(prev_o, NU - 1)
        return res + d, saved, filled

    def emit_out(r):
        xr = x_v[pl.ds(r, 2 * SEG), :].astype(_F32)
        gate = jax.nn.silu(gate_v[pl.ds(r, 2 * SEG), :])
        out_v[pl.ds(r, 2 * SEG), :] = (xr + s_v[...] * gate).astype(out_v.dtype)

    def out_copy(r):
        return pltpu.make_async_copy(out_v.at[pl.ds(r, 2 * SEG), :], out_hbm.at[pl.ds(r, 2 * SEG), :],
                                     sems.at[0])

    def pair_step(j, mem):
        r = pl.multiple_of(j * (2 * SEG), 2 * SEG)
        hb = jnp.concatenate([mem, xn_v[pl.ds(r, SEG + 8), :]], axis=0).astype(_BF16)
        extra = [None] * NU

        def fq_a(u, raw):
            extra[u] = tuple(t[L:] for t in raw)
            return tuple(t[:L] for t in raw)

        def fo_a(u, o):
            return o[:SEG], o[SEG:]

        c = NC - 1
        xb = xn_v[pl.ds(r, 2 * SEG), :].astype(_BF16)

        def fill_a():
            return jnp.dot(xb, _as_bf16(wg_v[:, c * FC:(c + 1) * FC]), preferred_element_type=_F32)

        res_a, tail_o, g = half(hb, fq_a, fo_a, fill_a)
        u_ = jnp.dot(xb, _as_bf16(wu_v[:, c * FC:(c + 1) * FC]), preferred_element_type=_F32)
        hh = (jax.nn.sigmoid(g) * u_).astype(_BF16)
        mem = res_a[:M]
        rp = pl.multiple_of(jnp.maximum(j - 1, 0) * (2 * SEG), 2 * SEG)
        emit_out(rp)
        hb = jnp.concatenate([mem, xn_v[pl.ds(r + SEG + 8, SEG - 8), :]], axis=0).astype(_BF16)

        def fq_b(u, raw):
            return tuple(jnp.concatenate([t[:M], ex, t[M:]], axis=0) for t, ex in zip(raw, extra[u]))

        def fo_b(u, o):
            return jnp.concatenate([o[:M], tail_o[u], o[M:]], axis=0), None

        def fill_b():
            return jnp.dot(hh, _as_bf16(wd_v[c * (FC // 2):(c + 1) * (FC // 2), :]),
                           preferred_element_type=_F32)

        res_b, _, d = half(hb, fq_b, fo_b, fill_b)
        gate_v[pl.ds(r, 2 * SEG), :] += d
        s_v[:SEG - 8, :] = res_a[M:]
        s_v[SEG - 8:, :] = res_b[M:]

        @pl.when(j > 0)
        def _():
            out_copy(rp).start()

        return res_b[:M]

    jax.lax.fori_loop(0, n_seg // 2, pair_step, mem0_ref[...].astype(_F32))
    r_last = S - 2 * SEG
    emit_out(r_last)
    out_copy(r_last).start()

    pltpu.make_async_copy(out_v, out_hbm, sems.at[0]).wait()


@functools.partial(jax.jit, static_argnames=("A_seg_len",))
def pallas_recurrent_scan__memory_aug_recurrent_mem_tr__glu_gated_glu__prompt_kernel(
    A_x: jax.Array,
    A_mem0: jax.Array,
    A_Wq: jax.Array,
    A_Wk: jax.Array,
    A_Wv: jax.Array,
    A_Wo: jax.Array,
    A_seg_len: int,
    B_x: jax.Array,
    B_w_gate: jax.Array,
    B_w_up: jax.Array,
    B_w_down: jax.Array,
):
    del B_x
    B, S, D = A_x.shape
    _, H, E = A_Wq.shape
    M = A_mem0.shape[1]
    F = B_w_gate.shape[1]
    SEG = int(A_seg_len)
    assert B == 1 and S % SEG == 0

    kern = functools.partial(_kernel, S=S, D=D, H=H, E=E, M=M, SEG=SEG, F=F, MB=256, FC=512, HG=4)
    any_spec = pl.BlockSpec(memory_space=pl.ANY)
    out = pl.pallas_call(
        kern,
        out_shape=jax.ShapeDtypeStruct((S, D), A_x.dtype),
        in_specs=[any_spec, pl.BlockSpec(memory_space=pltpu.VMEM)] + [any_spec] * 7,
        out_specs=any_spec,
        scratch_shapes=[
            pltpu.VMEM((S, D), _BF16),
            pltpu.VMEM((S, D), _F32),
            pltpu.VMEM((S, D), _F32),
            pltpu.VMEM((S, D), _BF16),
            pltpu.VMEM((D // 2, H * E), _U32),
            pltpu.VMEM((D // 2, H * E), _U32),
            pltpu.VMEM((D // 2, H * E), _U32),
            pltpu.VMEM((H * E // 2, D), _U32),
            pltpu.VMEM((D // 2, F), _U32),
            pltpu.VMEM((D // 2, F), _U32),
            pltpu.VMEM((F // 2, D), _U32),
            pltpu.VMEM((2, 2, H // 2, D // 2, E), _U32),
            pltpu.VMEM((2 * SEG, D), _F32),
            pltpu.VMEM((2, 5, D // 4, 512), _U32),
            pltpu.VMEM((2, 5, 128, D // 2), _U32),
            pltpu.SemaphoreType.DMA((4 + F // 512,)),
        ],
        compiler_params=pltpu.CompilerParams(vmem_limit_bytes=120 * 1024 * 1024),
    )(
        A_x.reshape(S, D),
        A_mem0.reshape(M, D),
        A_Wq.reshape(D // 2, 2, H, E),
        A_Wk.reshape(D // 2, 2, H, E),
        A_Wv.reshape(D // 2, 2, H, E),
        A_Wo.reshape(H * E, D),
        B_w_gate,
        B_w_up,
        B_w_down,
    )
    return out.reshape(B, S, D)
```

```python
import functools

import jax
import jax.numpy as jnp
import numpy as np
import jax.experimental.pallas as pl
import jax.experimental.pallas.tpu as pltpu

_F32 = jnp.float32
_BF16 = jnp.bfloat16
_U32 = jnp.uint32


def _as_bf16(w_u32):
    return pltpu.bitcast(w_u32, _BF16)


def _kernel(x_hbm, mem0_ref, wq_hbm, wk_hbm, wv_hbm, wo_hbm, wg_hbm, wu_hbm, wd_hbm,
            out_hbm,
            x_v, xn_v, gate_v, out_v, wq_v, wk_v, wv_v, wo_v, wg_v, wu_v, wd_v, st_v, s_v, sg_v, sd_v,
            sems,
            *, S, D, H, E, M, SEG, F, MB, FC, HG):
    n_seg = S // SEG
    scale = E ** (-0.5)
    L = M + SEG

    NC = F // FC
    NB = S // MB
    H2 = H // 2
    cp_x0 = pltpu.make_async_copy(x_hbm.at[pl.ds(0, MB)], x_v.at[pl.ds(0, MB)], sems.at[0])
    XS = S // 2 + MB
    cp_x = pltpu.make_async_copy(x_hbm.at[pl.ds(MB, XS - MB)], x_v.at[pl.ds(MB, XS - MB)], sems.at[2])
    cp_x2 = pltpu.make_async_copy(x_hbm.at[pl.ds(XS, S - XS)], x_v.at[pl.ds(XS, S - XS)], sems.at[3])
    cp_o = pltpu.make_async_copy(wo_hbm.bitcast(_U32), wo_v, sems.at[1])

    def chunk_copies(c):
        return [
            pltpu.make_async_copy(wg_hbm.bitcast(_U32).at[:, pl.ds(c * FC, FC)],
                                  wg_v.at[:, pl.ds(c * FC, FC)], sems.at[4 + c]),
            pltpu.make_async_copy(wu_hbm.bitcast(_U32).at[:, pl.ds(c * FC, FC)],
                                  wu_v.at[:, pl.ds(c * FC, FC)], sems.at[4 + c]),
            pltpu.make_async_copy(wd_hbm.bitcast(_U32).at[pl.ds(c * (FC // 2), FC // 2), :],
                                  wd_v.at[pl.ds(c * (FC // 2), FC // 2), :], sems.at[4 + c]),
        ]

    def gather_copies(w_hbm, slot):
        wu = w_hbm.bitcast(_U32)
        return [pltpu.make_async_copy(wu.at[:, p, h2, :], st_v.at[slot, p, h2], sems.at[2 + slot])
                for p in range(2) for h2 in range(H2)]

    def start(cs):
        for c in cs:
            c.start()

    def wait(cs):
        for c in cs:
            c.wait()

    def repack(slot, dst, h2):
        a = st_v[slot, 0, h2]
        b = st_v[slot, 1, h2]
        lo = (a & 0xFFFF) | (b << 16)
        hi = (a >> 16) | (b & np.uint32(0xFFFF0000))
        c0 = pl.multiple_of(h2 * (2 * E), 2 * E)
        dst[:, pl.ds(c0, E)] = lo
        dst[:, pl.ds(c0 + E, E)] = hi

    def layernorm(i):
        r = pl.multiple_of(i * MB, MB)
        xv = x_v[pl.ds(r, MB), :].astype(_F32)
        mu = jnp.mean(xv, axis=-1, keepdims=True)
        xc = xv - mu
        var = jnp.mean(xc * xc, axis=-1, keepdims=True)
        xn_v[pl.ds(r, MB), :] = xc / jnp.sqrt(var + 1e-5)

    KH, FH, DH, MH = D // 4, FC // 4, D // 2, MB // 2

    def w_blocks(c, lo, n, lo2, n2):
        return ((wg_v[pl.ds(lo, n), c * FC:(c + 1) * FC], wu_v[pl.ds(lo, n), c * FC:(c + 1) * FC],
                 wg_v[pl.ds(KH + lo, n), c * FC:(c + 1) * FC], wu_v[pl.ds(KH + lo, n), c * FC:(c + 1) * FC]),
                (wd_v[pl.ds(2 * c * FH + lo2, n2), :DH], wd_v[pl.ds(2 * c * FH + lo2, n2), DH:],
                 wd_v[pl.ds((2 * c + 1) * FH + lo2, n2), :DH], wd_v[pl.ds((2 * c + 1) * FH + lo2, n2), DH:]))

    def w_sums(b):
        w11, w12, w21, w22 = (_as_bf16(t).astype(_F32) for t in b)
        return [pltpu.bitcast(t.astype(_BF16), _U32)
                for t in (w11 + w22, w12 - w22, w21 - w11, w11 + w12, w21 + w22)]

    def prep(c, i):
        n, n2 = KH // NB, FH // NB
        lo, lo2 = pl.multiple_of(i * n, n), pl.multiple_of(i * n2, n2)
        gu, dn = w_blocks(c, lo, n, lo2, n2)
        for t, v in enumerate(w_sums(gu)):
            sg_v[c % 2, t, pl.ds(lo, n), :] = v
        for t, v in enumerate(w_sums(dn)):
            sd_v[c % 2, t, pl.ds(lo2, n2), :] = v

    def mm(l, w):
        return jnp.dot(l.astype(_BF16), _as_bf16(w), preferred_element_type=_F32)

    def acc(c, rows, cols, v):
        if c == 0:
            gate_v[rows, cols] = v
        else:
            gate_v[rows, cols] += v

    def glu_block_s(c, i):
        r = pl.multiple_of(i * MB, MB)
        r2 = pl.multiple_of(r + MH, MH)
        (w11, _, _, w22), (d11, _, _, d22) = w_blocks(c, 0, KH, 0, FH)
        sg = lambda t: sg_v[c % 2, t]
        sd = lambda t: sd_v[c % 2, t]
        a11, a12 = xn_v[pl.ds(r, MH), :DH], xn_v[pl.ds(r, MH), DH:]
        a21, a22 = xn_v[pl.ds(r2, MH), :DH], xn_v[pl.ds(r2, MH), DH:]
        m4 = mm(a22, sg(2))
        m1 = mm(a11 + a22, sg(0))
        m5 = mm(a11 + a12, w22)
        m7 = mm(a12 - a22, sg(4))
        g_top = m1 + m4 - m5 + m7
        m3 = mm(a11, sg(1))
        h_top = jax.nn.sigmoid(g_top) * (m3 + m5)
        m2 = mm(a21 + a22, w11)
        m6 = mm(a21 - a11, sg(3))
        h_bot = jax.nn.sigmoid(m2 + m4) * (m1 - m2 + m3 + m6)
        FQ = FC // 2
        b11, b12, b21, b22 = h_top[:, :FQ], h_top[:, FQ:], h_bot[:, :FQ], h_bot[:, FQ:]
        n3 = mm(b11, sd(1))
        n5 = mm(b11 + b12, d22)
        acc(c, pl.ds(r, MH), slice(DH, D), n3 + n5)
        n1 = mm(b11 + b22, sd(0))
        n4 = mm(b22, sd(2))
        n7 = mm(b12 - b22, sd(4))
        acc(c, pl.ds(r, MH), slice(0, DH), n1 + n4 - n5 + n7)
        n2 = mm(b21 + b22, d11)
        acc(c, pl.ds(r2, MH), slice(0, DH), n2 + n4)
        n6 = mm(b21 - b11, sd(3))
        acc(c, pl.ds(r2, MH), slice(DH, D), n1 - n2 + n3 + n6)

    def glu_chunk(c, side=None, lo=0, hi=None, do_prep=True):
        @pl.loop(lo, NB if hi is None else hi)
        def _(i):
            glu_block_s(c, i)
            if do_prep and c + 1 < NC - 1:
                prep(c + 1, i)
            if side is not None:
                side(i)

    per = H2 // NB
    cp_x0.start()
    start(chunk_copies(0))
    cp_x.start()
    cp_x0.wait()
    layernorm(0)
    wait(chunk_copies(0))
    cp_x2.start()
    for c in range(1, NC):
        start(chunk_copies(c))
    cp_o.start()
    pl.loop(0, NB)(lambda i: prep(0, i))
    cp_x.wait()
    ln_next = lambda i: layernorm(jnp.minimum(i + 1, NB - 1))
    glu_chunk(0, ln_next, hi=NB // 2, do_prep=False)
    wait(chunk_copies(1))
    cp_x2.wait()

    def side0(i):
        ln_next(i)
        prep(1, 2 * i - NB)
        prep(1, 2 * i - NB + 1)

    glu_chunk(0, side0, lo=NB // 2, do_prep=False)
    for c in range(2, NC - 1):
        wait(chunk_copies(c))
    start(gather_copies(wq_hbm, 0))
    start(gather_copies(wk_hbm, 1))
    glu_chunk(1)
    wait(gather_copies(wq_hbm, 0))

    def side_repack(slot, dst):
        def f(i):
            for t in range(per):
                repack(slot, dst, i * per + t)
        return f

    glu_chunk(2, side_repack(0, wq_v))
    start(gather_copies(wv_hbm, 0))
    wait(gather_copies(wk_hbm, 1))
    glu_chunk(3, side_repack(1, wk_v))
    glu_chunk(4)
    wait(gather_copies(wv_hbm, 0))
    glu_chunk(5, side_repack(0, wv_v))
    for c in range(6, NC - 1):
        glu_chunk(c)
    wait(chunk_copies(NC - 1))
    cp_o.wait()
    s_v[...] = jnp.zeros_like(s_v)

    row = jax.lax.broadcasted_iota(jnp.int32, (2 * L, 2 * L), 0)
    col = jax.lax.broadcasted_iota(jnp.int32, (2 * L, 2 * L), 1)
    r_in = jnp.where(row >= L, row - L, row)
    c_in = jnp.where(col >= L, col - L, col)
    mask = ((row >= L) == (col >= L)) & ((r_in < M) | (r_in >= c_in))
    NU = H // 2
    UW = 2 * E

    def qkv(hb, u):
        return tuple(
            jnp.dot(hb, _as_bf16(w[:, u * UW:(u + 1) * UW]), preferred_element_type=_F32)
            for w in (wq_v, wk_v, wv_v))

    def stack(t):
        return jnp.concatenate([t[:, :E], t[:, E:]], axis=0).astype(_BF16)

    def scores(q, k):
        sc = jax.lax.dot_general(stack(q), stack(k), (((1,), (1,)), ((), ())),
                                 preferred_element_type=_F32) * scale
        sc = jnp.where(mask, sc, -1e9)
        e = jnp.exp(sc - jnp.max(sc, axis=-1, keepdims=True))
        return (e / jnp.sum(e, axis=-1, keepdims=True)).astype(_BF16)

    def pv(p, v):
        o = jnp.dot(p, stack(v), preferred_element_type=_F32)
        return jnp.concatenate([o[:L], o[L:]], axis=1)

    def proj(o, u):
        return jnp.dot(o.astype(_BF16), _as_bf16(wo_v[u * E:(u + 1) * E, :]),
                       preferred_element_type=_F32)

    def half(hb, fix_qkv, fix_o, fill):
        res = None
        saved = [None] * NU
        raw = qkv(hb, 0)
        prev_o = None
        for u in range(NU):
            q, k, v = fix_qkv(u, raw)
            p = scores(q, k)
            if u + 1 < NU:
                raw = qkv(hb, u + 1)
            elif prev_o is not None:
                d = proj(prev_o, u - 1)
                res = d if res is None else res + d
                prev_o = None
            o = pv(p, v)
            if prev_o is not None:
                d = proj(prev_o, u - 1)
                res = d if res is None else res + d
            prev_o, saved[u] = fix_o(u, o)
        filled = fill()
        d = proj(prev_o, NU - 1)
        return res + d, saved, filled

    def emit_out(r):
        xr = x_v[pl.ds(r, 2 * SEG), :].astype(_F32)
        gate = jax.nn.silu(gate_v[pl.ds(r, 2 * SEG), :])
        out_v[pl.ds(r, 2 * SEG), :] = (xr + s_v[...] * gate).astype(out_v.dtype)

    def out_copy(r):
        return pltpu.make_async_copy(out_v.at[pl.ds(r, 2 * SEG), :], out_hbm.at[pl.ds(r, 2 * SEG), :],
                                     sems.at[0])

    def pair_step(j, mem):
        r = pl.multiple_of(j * (2 * SEG), 2 * SEG)
        hb = jnp.concatenate([mem, xn_v[pl.ds(r, SEG + 8), :]], axis=0).astype(_BF16)
        extra = [None] * NU

        def fq_a(u, raw):
            extra[u] = tuple(t[L:] for t in raw)
            return tuple(t[:L] for t in raw)

        def fo_a(u, o):
            return o[:SEG], o[SEG:]

        c = NC - 1
        xb = xn_v[pl.ds(r, 2 * SEG), :].astype(_BF16)

        def fill_a():
            return jnp.dot(xb, _as_bf16(wg_v[:, c * FC:(c + 1) * FC]), preferred_element_type=_F32)

        res_a, tail_o, g = half(hb, fq_a, fo_a, fill_a)
        u_ = jnp.dot(xb, _as_bf16(wu_v[:, c * FC:(c + 1) * FC]), preferred_element_type=_F32)
        hh = (jax.nn.sigmoid(g) * u_).astype(_BF16)
        mem = res_a[:M]
        rp = pl.multiple_of(jnp.maximum(j - 1, 0) * (2 * SEG), 2 * SEG)
        emit_out(rp)
        hb = jnp.concatenate([mem, xn_v[pl.ds(r + SEG + 8, SEG - 8), :]], axis=0).astype(_BF16)

        def fq_b(u, raw):
            return tuple(jnp.concatenate([t[:M], ex, t[M:]], axis=0) for t, ex in zip(raw, extra[u]))

        def fo_b(u, o):
            return jnp.concatenate([o[:M], tail_o[u], o[M:]], axis=0), None

        def fill_b():
            return jnp.dot(hh, _as_bf16(wd_v[c * (FC // 2):(c + 1) * (FC // 2), :]),
                           preferred_element_type=_F32)

        res_b, _, d = half(hb, fq_b, fo_b, fill_b)
        gate_v[pl.ds(r, 2 * SEG), :] += d
        s_v[:SEG - 8, :] = res_a[M:]
        s_v[SEG - 8:, :] = res_b[M:]

        @pl.when(j > 0)
        def _():
            out_copy(rp).start()

        return res_b[:M]

    jax.lax.fori_loop(0, n_seg // 2, pair_step, mem0_ref[...].astype(_F32))
    r_last = S - 2 * SEG
    emit_out(r_last)
    out_copy(r_last).start()

    pltpu.make_async_copy(out_v, out_hbm, sems.at[0]).wait()


@functools.partial(jax.jit, static_argnames=("A_seg_len",))
def pallas_recurrent_scan__memory_aug_recurrent_mem_tr__glu_gated_glu__prompt_kernel(
    A_x: jax.Array,
    A_mem0: jax.Array,
    A_Wq: jax.Array,
    A_Wk: jax.Array,
    A_Wv: jax.Array,
    A_Wo: jax.Array,
    A_seg_len: int,
    B_x: jax.Array,
    B_w_gate: jax.Array,
    B_w_up: jax.Array,
    B_w_down: jax.Array,
):
    del B_x
    B, S, D = A_x.shape
    _, H, E = A_Wq.shape
    M = A_mem0.shape[1]
    F = B_w_gate.shape[1]
    SEG = int(A_seg_len)
    assert B == 1 and S % SEG == 0

    kern = functools.partial(_kernel, S=S, D=D, H=H, E=E, M=M, SEG=SEG, F=F, MB=256, FC=512, HG=4)
    any_spec = pl.BlockSpec(memory_space=pl.ANY)
    out = pl.pallas_call(
        kern,
        out_shape=jax.ShapeDtypeStruct((S, D), A_x.dtype),
        in_specs=[any_spec, pl.BlockSpec(memory_space=pltpu.VMEM)] + [any_spec] * 7,
        out_specs=any_spec,
        scratch_shapes=[
            pltpu.VMEM((S, D), _BF16),
            pltpu.VMEM((S, D), _F32),
            pltpu.VMEM((S, D), _F32),
            pltpu.VMEM((S, D), _BF16),
            pltpu.VMEM((D // 2, H * E), _U32),
            pltpu.VMEM((D // 2, H * E), _U32),
            pltpu.VMEM((D // 2, H * E), _U32),
            pltpu.VMEM((H * E // 2, D), _U32),
            pltpu.VMEM((D // 2, F), _U32),
            pltpu.VMEM((D // 2, F), _U32),
            pltpu.VMEM((F // 2, D), _U32),
            pltpu.VMEM((2, 2, H // 2, D // 2, E), _U32),
            pltpu.VMEM((2 * SEG, D), _F32),
            pltpu.VMEM((2, 5, D // 4, 512), _U32),
            pltpu.VMEM((2, 5, 128, D // 2), _U32),
            pltpu.SemaphoreType.DMA((4 + F // 512,)),
        ],
        compiler_params=pltpu.CompilerParams(vmem_limit_bytes=120 * 1024 * 1024),
    )(
        A_x.reshape(S, D),
        A_mem0.reshape(M, D),
        A_Wq.reshape(D // 2, 2, H, E),
        A_Wk.reshape(D // 2, 2, H, E),
        A_Wv.reshape(D // 2, 2, H, E),
        A_Wo.reshape(H * E, D),
        B_w_gate,
        B_w_up,
        B_w_down,
    )
    return out.reshape(B, S, D)
```

```python
import functools

import jax
import jax.numpy as jnp
import numpy as np
import jax.experimental.pallas as pl
import jax.experimental.pallas.tpu as pltpu

_F32 = jnp.float32
_BF16 = jnp.bfloat16
_U32 = jnp.uint32


def _as_bf16(w_u32):
    return pltpu.bitcast(w_u32, _BF16)


def _kernel(x_hbm, mem0_ref, wq_hbm, wk_hbm, wv_hbm, wo_hbm, wg_hbm, wu_hbm, wd_hbm,
            out_hbm,
            x_v, xn_v, gate_v, out_v, wq_v, wk_v, wv_v, wo_v, wg_v, wu_v, wd_v, st_v, s_v, sg_v, sd_v,
            sems,
            *, S, D, H, E, M, SEG, F, MB, FC, HG):
    n_seg = S // SEG
    scale = E ** (-0.5)
    L = M + SEG

    NC = F // FC
    NB = S // MB
    H2 = H // 2
    cp_x0 = pltpu.make_async_copy(x_hbm.at[pl.ds(0, MB)], x_v.at[pl.ds(0, MB)], sems.at[0])
    XS = S // 2 + MB
    cp_x = pltpu.make_async_copy(x_hbm.at[pl.ds(MB, XS - MB)], x_v.at[pl.ds(MB, XS - MB)], sems.at[2])
    cp_x2 = pltpu.make_async_copy(x_hbm.at[pl.ds(XS, S - XS)], x_v.at[pl.ds(XS, S - XS)], sems.at[3])
    cp_o = pltpu.make_async_copy(wo_hbm.bitcast(_U32), wo_v, sems.at[1])

    def chunk_copies(c):
        return [
            pltpu.make_async_copy(wg_hbm.bitcast(_U32).at[:, pl.ds(c * FC, FC)],
                                  wg_v.at[:, pl.ds(c * FC, FC)], sems.at[4 + c]),
            pltpu.make_async_copy(wu_hbm.bitcast(_U32).at[:, pl.ds(c * FC, FC)],
                                  wu_v.at[:, pl.ds(c * FC, FC)], sems.at[4 + c]),
            pltpu.make_async_copy(wd_hbm.bitcast(_U32).at[pl.ds(c * (FC // 2), FC // 2), :],
                                  wd_v.at[pl.ds(c * (FC // 2), FC // 2), :], sems.at[4 + c]),
        ]

    def gather_copies(w_hbm, slot):
        wu = w_hbm.bitcast(_U32)
        return [pltpu.make_async_copy(wu.at[:, p, h2, :], st_v.at[slot, p, h2], sems.at[2 + slot])
                for p in range(2) for h2 in range(H2)]

    def start(cs):
        for c in cs:
            c.start()

    def wait(cs):
        for c in cs:
            c.wait()

    def repack(slot, dst, h2):
        a = st_v[slot, 0, h2]
        b = st_v[slot, 1, h2]
        lo = (a & 0xFFFF) | (b << 16)
        hi = (a >> 16) | (b & np.uint32(0xFFFF0000))
        c0 = pl.multiple_of(h2 * (2 * E), 2 * E)
        dst[:, pl.ds(c0, E)] = lo
        dst[:, pl.ds(c0 + E, E)] = hi

    def layernorm(i):
        r = pl.multiple_of(i * MB, MB)
        xv = x_v[pl.ds(r, MB), :].astype(_F32)
        mu = jnp.mean(xv, axis=-1, keepdims=True)
        xc = xv - mu
        var = jnp.mean(xc * xc, axis=-1, keepdims=True)
        xn_v[pl.ds(r, MB), :] = xc / jnp.sqrt(var + 1e-5)

    KH, FH, DH, MH = D // 4, FC // 4, D // 2, MB // 2

    def w_blocks(c, lo, n, lo2, n2):
        return ((wg_v[pl.ds(lo, n), c * FC:(c + 1) * FC], wu_v[pl.ds(lo, n), c * FC:(c + 1) * FC],
                 wg_v[pl.ds(KH + lo, n), c * FC:(c + 1) * FC], wu_v[pl.ds(KH + lo, n), c * FC:(c + 1) * FC]),
                (wd_v[pl.ds(2 * c * FH + lo2, n2), :DH], wd_v[pl.ds(2 * c * FH + lo2, n2), DH:],
                 wd_v[pl.ds((2 * c + 1) * FH + lo2, n2), :DH], wd_v[pl.ds((2 * c + 1) * FH + lo2, n2), DH:]))

    def w_sums(b):
        w11, w12, w21, w22 = (_as_bf16(t).astype(_F32) for t in b)
        return [pltpu.bitcast(t.astype(_BF16), _U32)
                for t in (w11 + w22, w12 - w22, w21 - w11, w11 + w12, w21 + w22)]

    def prep(c, i):
        n, n2 = KH // NB, FH // NB
        lo, lo2 = pl.multiple_of(i * n, n), pl.multiple_of(i * n2, n2)
        gu, dn = w_blocks(c, lo, n, lo2, n2)
        for t, v in enumerate(w_sums(gu)):
            sg_v[c, t, pl.ds(lo, n), :] = v
        for t, v in enumerate(w_sums(dn)):
            sd_v[c, t, pl.ds(lo2, n2), :] = v

    def mm(l, w):
        return jnp.dot(l.astype(_BF16), _as_bf16(w), preferred_element_type=_F32)

    def acc(c, rows, cols, v):
        if c == 0:
            gate_v[rows, cols] = v
        else:
            gate_v[rows, cols] += v

    def glu_gen(c, r, MH):
        r2 = pl.multiple_of(r + MH, MH)
        (w11, _, _, w22), (d11, _, _, d22) = w_blocks(c, 0, KH, 0, FH)
        sg = lambda t: sg_v[c, t]
        sd = lambda t: sd_v[c, t]
        a11, a12 = xn_v[pl.ds(r, MH), :DH], xn_v[pl.ds(r, MH), DH:]
        a21, a22 = xn_v[pl.ds(r2, MH), :DH], xn_v[pl.ds(r2, MH), DH:]
        m4 = mm(a22, sg(2))
        yield
        m1 = mm(a11 + a22, sg(0))
        yield
        m5 = mm(a11 + a12, w22)
        yield
        m7 = mm(a12 - a22, sg(4))
        yield
        g_top = m1 + m4 - m5 + m7
        m3 = mm(a11, sg(1))
        yield
        h_top = jax.nn.sigmoid(g_top) * (m3 + m5)
        m2 = mm(a21 + a22, w11)
        yield
        m6 = mm(a21 - a11, sg(3))
        yield
        h_bot = jax.nn.sigmoid(m2 + m4) * (m1 - m2 + m3 + m6)
        FQ = FC // 2
        b11, b12, b21, b22 = h_top[:, :FQ], h_top[:, FQ:], h_bot[:, :FQ], h_bot[:, FQ:]
        n3 = mm(b11, sd(1))
        yield
        n5 = mm(b11 + b12, d22)
        yield
        acc(c, pl.ds(r, MH), slice(DH, D), n3 + n5)
        n1 = mm(b11 + b22, sd(0))
        yield
        n4 = mm(b22, sd(2))
        yield
        n7 = mm(b12 - b22, sd(4))
        yield
        acc(c, pl.ds(r, MH), slice(0, DH), n1 + n4 - n5 + n7)
        n2 = mm(b21 + b22, d11)
        yield
        acc(c, pl.ds(r2, MH), slice(0, DH), n2 + n4)
        n6 = mm(b21 - b11, sd(3))
        yield
        acc(c, pl.ds(r2, MH), slice(DH, D), n1 - n2 + n3 + n6)

    def glu_block_s(c, i):
        for _ in glu_gen(c, pl.multiple_of(i * MB, MB), MH):
            pass

    CB = 3
    NH = NB // 2

    def glu_half(c, h, side):
        @pl.loop(h * NH, (h + 1) * NH)
        def _(i):
            glu_block_s(c, i)
            side(i - h * NH)

    def preps(c, i):
        prep(c, 2 * i)
        prep(c, 2 * i + 1)

    def repacks(slot, dst, i):
        per = H2 // NH
        for t in range(per):
            repack(slot, dst, i * per + t)

    cp_x0.start()
    start(chunk_copies(0))
    cp_x.start()
    cp_x0.wait()
    layernorm(0)
    wait(chunk_copies(0))
    cp_x2.start()
    start(chunk_copies(1))
    start(chunk_copies(2))
    pl.loop(0, NB)(lambda i: prep(0, i))
    cp_x.wait()
    glu_half(0, 0, lambda i: layernorm(i + 1))
    start(gather_copies(wq_hbm, 0))
    for c in range(CB, NC):
        start(chunk_copies(c))
    wait(chunk_copies(1))
    cp_x2.wait()

    def side(i):
        layernorm(jnp.minimum(NH + i + 1, NB - 1))
        preps(1, i)

    glu_half(0, 1, side)
    start(gather_copies(wk_hbm, 1))
    cp_o.start()
    wait(chunk_copies(2))
    glu_half(1, 0, lambda i: preps(2, i))
    wait(gather_copies(wq_hbm, 0))
    for c in range(CB, NC):
        wait(chunk_copies(c))

    def side(i):
        repacks(0, wq_v, i)
        preps(3, i)

    glu_half(1, 1, side)
    start(gather_copies(wv_hbm, 0))
    wait(gather_copies(wk_hbm, 1))

    def side(i):
        repacks(1, wk_v, i)
        preps(4, i)
        preps(5, i)

    glu_half(2, 0, side)
    wait(gather_copies(wv_hbm, 0))

    def side(i):
        repacks(0, wv_v, i)
        preps(6, i)

    glu_half(2, 1, side)
    cp_o.wait()
    s_v[...] = jnp.zeros_like(s_v)

    row = jax.lax.broadcasted_iota(jnp.int32, (2 * L, 2 * L), 0)
    col = jax.lax.broadcasted_iota(jnp.int32, (2 * L, 2 * L), 1)
    r_in = jnp.where(row >= L, row - L, row)
    c_in = jnp.where(col >= L, col - L, col)
    mask = ((row >= L) == (col >= L)) & ((r_in < M) | (r_in >= c_in))
    NU = H // 2
    UW = 2 * E

    def qkv(hb, u):
        return tuple(
            jnp.dot(hb, _as_bf16(w[:, u * UW:(u + 1) * UW]), preferred_element_type=_F32)
            for w in (wq_v, wk_v, wv_v))

    def stack(t):
        return jnp.concatenate([t[:, :E], t[:, E:]], axis=0).astype(_BF16)

    def scores(q, k):
        sc = jax.lax.dot_general(stack(q), stack(k), (((1,), (1,)), ((), ())),
                                 preferred_element_type=_F32) * scale
        sc = jnp.where(mask, sc, -1e9)
        e = jnp.exp(sc - jnp.max(sc, axis=-1, keepdims=True))
        return (e / jnp.sum(e, axis=-1, keepdims=True)).astype(_BF16)

    def pv(p, v):
        o = jnp.dot(p, stack(v), preferred_element_type=_F32)
        return jnp.concatenate([o[:L], o[L:]], axis=1)

    def proj(o, u):
        return jnp.dot(o.astype(_BF16), _as_bf16(wo_v[u * E:(u + 1) * E, :]),
                       preferred_element_type=_F32)

    def half(hb, fix_qkv, fix_o, fill):
        res = None
        saved = [None] * NU
        raw = qkv(hb, 0)
        prev_o = None
        for u in range(NU):
            q, k, v = fix_qkv(u, raw)
            p = scores(q, k)
            if u + 1 < NU:
                raw = qkv(hb, u + 1)
            elif prev_o is not None:
                d = proj(prev_o, u - 1)
                res = d if res is None else res + d
                prev_o = None
            fill()
            o = pv(p, v)
            if prev_o is not None:
                d = proj(prev_o, u - 1)
                res = d if res is None else res + d
            prev_o, saved[u] = fix_o(u, o)
        fill()
        fill()
        d = proj(prev_o, NU - 1)
        return res + d, saved

    def emit_out(r):
        xr = x_v[pl.ds(r, 2 * SEG), :].astype(_F32)
        gate = jax.nn.silu(gate_v[pl.ds(r, 2 * SEG), :])
        out_v[pl.ds(r, 2 * SEG), :] = (xr + s_v[...] * gate).astype(out_v.dtype)

    def out_copy(r):
        return pltpu.make_async_copy(out_v.at[pl.ds(r, 2 * SEG), :], out_hbm.at[pl.ds(r, 2 * SEG), :],
                                     sems.at[0])

    def pair_step(j, mem):
        r = pl.multiple_of(j * (2 * SEG), 2 * SEG)
        hb = jnp.concatenate([mem, xn_v[pl.ds(r, SEG + 8), :]], axis=0).astype(_BF16)
        extra = [None] * NU

        def fq_a(u, raw):
            extra[u] = tuple(t[L:] for t in raw)
            return tuple(t[:L] for t in raw)

        def fo_a(u, o):
            return o[:SEG], o[SEG:]

        def glu_all():
            for c in range(CB, NC):
                yield from glu_gen(c, r, SEG)

        gen = glu_all()
        fill = lambda: next(gen, None)
        res_a, tail_o = half(hb, fq_a, fo_a, fill)
        fill()
        fill()
        mem = res_a[:M]
        rp = pl.multiple_of(jnp.maximum(j - 1, 0) * (2 * SEG), 2 * SEG)
        emit_out(rp)
        hb = jnp.concatenate([mem, xn_v[pl.ds(r + SEG + 8, SEG - 8), :]], axis=0).astype(_BF16)

        def fq_b(u, raw):
            return tuple(jnp.concatenate([t[:M], ex, t[M:]], axis=0) for t, ex in zip(raw, extra[u]))

        def fo_b(u, o):
            return jnp.concatenate([o[:M], tail_o[u], o[M:]], axis=0), None

        res_b, _ = half(hb, fq_b, fo_b, fill)
        for _ in gen:
            pass
        s_v[:SEG - 8, :] = res_a[M:]
        s_v[SEG - 8:, :] = res_b[M:]

        @pl.when(j > 0)
        def _():
            out_copy(rp).start()

        return res_b[:M]

    jax.lax.fori_loop(0, n_seg // 2, pair_step, mem0_ref[...].astype(_F32))
    r_last = S - 2 * SEG
    emit_out(r_last)
    out_copy(r_last).start()

    pltpu.make_async_copy(out_v, out_hbm, sems.at[0]).wait()


@functools.partial(jax.jit, static_argnames=("A_seg_len",))
def pallas_recurrent_scan__memory_aug_recurrent_mem_tr__glu_gated_glu__prompt_kernel(
    A_x: jax.Array,
    A_mem0: jax.Array,
    A_Wq: jax.Array,
    A_Wk: jax.Array,
    A_Wv: jax.Array,
    A_Wo: jax.Array,
    A_seg_len: int,
    B_x: jax.Array,
    B_w_gate: jax.Array,
    B_w_up: jax.Array,
    B_w_down: jax.Array,
):
    del B_x
    B, S, D = A_x.shape
    _, H, E = A_Wq.shape
    M = A_mem0.shape[1]
    F = B_w_gate.shape[1]
    SEG = int(A_seg_len)
    assert B == 1 and S % SEG == 0

    kern = functools.partial(_kernel, S=S, D=D, H=H, E=E, M=M, SEG=SEG, F=F, MB=256, FC=512, HG=4)
    any_spec = pl.BlockSpec(memory_space=pl.ANY)
    out = pl.pallas_call(
        kern,
        out_shape=jax.ShapeDtypeStruct((S, D), A_x.dtype),
        in_specs=[any_spec, pl.BlockSpec(memory_space=pltpu.VMEM)] + [any_spec] * 7,
        out_specs=any_spec,
        scratch_shapes=[
            pltpu.VMEM((S, D), _BF16),
            pltpu.VMEM((S, D), _F32),
            pltpu.VMEM((S, D), _F32),
            pltpu.VMEM((S, D), _BF16),
            pltpu.VMEM((D // 2, H * E), _U32),
            pltpu.VMEM((D // 2, H * E), _U32),
            pltpu.VMEM((D // 2, H * E), _U32),
            pltpu.VMEM((H * E // 2, D), _U32),
            pltpu.VMEM((D // 2, F), _U32),
            pltpu.VMEM((D // 2, F), _U32),
            pltpu.VMEM((F // 2, D), _U32),
            pltpu.VMEM((2, 2, H // 2, D // 2, E), _U32),
            pltpu.VMEM((2 * SEG, D), _F32),
            pltpu.VMEM((F // 512, 5, D // 4, 512), _U32),
            pltpu.VMEM((F // 512, 5, 128, D // 2), _U32),
            pltpu.SemaphoreType.DMA((4 + F // 512,)),
        ],
        compiler_params=pltpu.CompilerParams(vmem_limit_bytes=127 * 1024 * 1024),
    )(
        A_x.reshape(S, D),
        A_mem0.reshape(M, D),
        A_Wq.reshape(D // 2, 2, H, E),
        A_Wk.reshape(D // 2, 2, H, E),
        A_Wv.reshape(D // 2, 2, H, E),
        A_Wo.reshape(H * E, D),
        B_w_gate,
        B_w_up,
        B_w_down,
    )
    return out.reshape(B, S, D)
```

```python
import functools

import jax
import jax.numpy as jnp
import numpy as np
import jax.experimental.pallas as pl
import jax.experimental.pallas.tpu as pltpu

_F32 = jnp.float32
_BF16 = jnp.bfloat16
_U32 = jnp.uint32


def _as_bf16(w_u32):
    return pltpu.bitcast(w_u32, _BF16)


def _kernel(x_hbm, mem0_ref, wq_hbm, wk_hbm, wv_hbm, wo_hbm, wg_hbm, wu_hbm, wd_hbm,
            out_hbm,
            x_v, xn_v, gate_v, out_v, wq_v, wk_v, wv_v, wo_v, wg_v, wu_v, wd_v, st_v, s_v, sg_v, sd_v,
            sems,
            *, S, D, H, E, M, SEG, F, MB, FC, HG):
    n_seg = S // SEG
    scale = E ** (-0.5)
    L = M + SEG

    NC = F // FC
    NB = S // MB
    H2 = H // 2
    cp_x0 = pltpu.make_async_copy(x_hbm.at[pl.ds(0, MB)], x_v.at[pl.ds(0, MB)], sems.at[0])
    XS = S // 2 + MB
    cp_x = pltpu.make_async_copy(x_hbm.at[pl.ds(MB, XS - MB)], x_v.at[pl.ds(MB, XS - MB)], sems.at[2])
    cp_x2 = pltpu.make_async_copy(x_hbm.at[pl.ds(XS, S - XS)], x_v.at[pl.ds(XS, S - XS)], sems.at[3])
    cp_o = pltpu.make_async_copy(wo_hbm.bitcast(_U32), wo_v, sems.at[1])

    def chunk_copies(c):
        return [
            pltpu.make_async_copy(wg_hbm.bitcast(_U32).at[:, pl.ds(c * FC, FC)],
                                  wg_v.at[:, pl.ds(c * FC, FC)], sems.at[4 + c]),
            pltpu.make_async_copy(wu_hbm.bitcast(_U32).at[:, pl.ds(c * FC, FC)],
                                  wu_v.at[:, pl.ds(c * FC, FC)], sems.at[4 + c]),
            pltpu.make_async_copy(wd_hbm.bitcast(_U32).at[pl.ds(c * (FC // 2), FC // 2), :],
                                  wd_v.at[pl.ds(c * (FC // 2), FC // 2), :], sems.at[4 + c]),
        ]

    def gather_copies(w_hbm, slot):
        wu = w_hbm.bitcast(_U32)
        return [pltpu.make_async_copy(wu.at[:, p, h2, :], st_v.at[slot, p, h2], sems.at[2 + slot])
                for p in range(2) for h2 in range(H2)]

    def start(cs):
        for c in cs:
            c.start()

    def wait(cs):
        for c in cs:
            c.wait()

    def repack(slot, dst, h2):
        a = st_v[slot, 0, h2]
        b = st_v[slot, 1, h2]
        lo = (a & 0xFFFF) | (b << 16)
        hi = (a >> 16) | (b & np.uint32(0xFFFF0000))
        c0 = pl.multiple_of(h2 * (2 * E), 2 * E)
        dst[:, pl.ds(c0, E)] = lo
        dst[:, pl.ds(c0 + E, E)] = hi

    def layernorm(i):
        r = pl.multiple_of(i * MB, MB)
        xv = x_v[pl.ds(r, MB), :].astype(_F32)
        mu = jnp.mean(xv, axis=-1, keepdims=True)
        xc = xv - mu
        var = jnp.mean(xc * xc, axis=-1, keepdims=True)
        xn_v[pl.ds(r, MB), :] = xc / jnp.sqrt(var + 1e-5)

    KH, FQ, FH, DH, MH = D // 4, FC // 2, FC // 4, D // 2, MB // 2

    def gu_blocks(w, c, lo, n):
        c0 = c * FC
        return (w[pl.ds(lo, n), c0:c0 + FQ], w[pl.ds(lo, n), c0 + FQ:c0 + FC],
                w[pl.ds(KH + lo, n), c0:c0 + FQ], w[pl.ds(KH + lo, n), c0 + FQ:c0 + FC])

    def dn_blocks(c, lo, n):
        r0 = 2 * c * FH
        return (wd_v[pl.ds(r0 + lo, n), :DH], wd_v[pl.ds(r0 + lo, n), DH:],
                wd_v[pl.ds(r0 + FH + lo, n), :DH], wd_v[pl.ds(r0 + FH + lo, n), DH:])

    def w_sums(b):
        w11, w12, w21, w22 = (_as_bf16(t).astype(_F32) for t in b)
        return [pltpu.bitcast(t.astype(_BF16), _U32)
                for t in (w11 + w22, w12 - w22, w21 - w11, w11 + w12, w21 + w22)]

    def prep(c, i):
        n, n2 = KH // NB, FH // NB
        lo, lo2 = pl.multiple_of(i * n, n), pl.multiple_of(i * n2, n2)
        for k, w in enumerate((wg_v, wu_v)):
            for t, v in enumerate(w_sums(gu_blocks(w, c, lo, n))):
                sg_v[c, t, pl.ds(lo, n), k * FQ:(k + 1) * FQ] = v
        for t, v in enumerate(w_sums(dn_blocks(c, lo2, n2))):
            sd_v[c, t, pl.ds(lo2, n2), :] = v

    def mm(l, w):
        return jnp.dot(l.astype(_BF16), _as_bf16(w), preferred_element_type=_F32)

    def acc(c, rows, cols, v):
        if c == 0:
            gate_v[rows, cols] = v
        else:
            gate_v[rows, cols] += v

    def glu_gen(c, r, MH):
        r2 = pl.multiple_of(r + MH, MH)
        g11, _, _, g22 = gu_blocks(wg_v, c, 0, KH)
        u11, _, _, u22 = gu_blocks(wu_v, c, 0, KH)
        w11 = jnp.concatenate([g11, u11], axis=1)
        w22 = jnp.concatenate([g22, u22], axis=1)
        d11, _, _, d22 = dn_blocks(c, 0, FH)
        sg = lambda t: sg_v[c, t]
        sd = lambda t: sd_v[c, t]
        glu = lambda z: jax.nn.sigmoid(z[:, :FQ]) * z[:, FQ:]
        a11, a12 = xn_v[pl.ds(r, MH), :DH], xn_v[pl.ds(r, MH), DH:]
        a21, a22 = xn_v[pl.ds(r2, MH), :DH], xn_v[pl.ds(r2, MH), DH:]
        m4 = mm(a22, sg(2))
        yield
        m1 = mm(a11 + a22, sg(0))
        yield
        m5 = mm(a11 + a12, w22)
        yield
        m7 = mm(a12 - a22, sg(4))
        yield
        b11 = glu(m1 + m4 - m5 + m7)
        m3 = mm(a11, sg(1))
        yield
        b12 = glu(m3 + m5)
        m2 = mm(a21 + a22, w11)
        yield
        b21 = glu(m2 + m4)
        m6 = mm(a21 - a11, sg(3))
        yield
        b22 = glu(m1 - m2 + m3 + m6)
        n3 = mm(b11, sd(1))
        yield
        n5 = mm(b11 + b12, d22)
        yield
        acc(c, pl.ds(r, MH), slice(DH, D), n3 + n5)
        n6 = mm(b21 - b11, sd(3))
        yield
        n1 = mm(b11 + b22, sd(0))
        yield
        n4 = mm(b22, sd(2))
        yield
        n7 = mm(b12 - b22, sd(4))
        yield
        acc(c, pl.ds(r, MH), slice(0, DH), n1 + n4 - n5 + n7)
        n2 = mm(b21 + b22, d11)
        yield
        acc(c, pl.ds(r2, MH), slice(0, DH), n2 + n4)
        acc(c, pl.ds(r2, MH), slice(DH, D), n1 - n2 + n3 + n6)

    CB = 3
    NH = NB // 2

    def glu_half(c, h, side):
        @pl.loop(h * NH, (h + 1) * NH)
        def _(i):
            todo = side(i - h * NH)
            for _ in glu_gen(c, pl.multiple_of(i * MB, MB), MH):
                if todo:
                    todo.pop(0)()
            for job in todo:
                job()

    def preps(c, i):
        return [functools.partial(prep, c, 2 * i + t) for t in range(2)]

    def repacks(slot, dst, i):
        per = H2 // NH
        return [functools.partial(repack, slot, dst, i * per + t) for t in range(per)]

    cp_x0.start()
    start(chunk_copies(0))
    cp_x.start()
    cp_x0.wait()
    layernorm(0)
    wait(chunk_copies(0))
    cp_x2.start()
    start(chunk_copies(1))
    start(chunk_copies(2))
    pl.loop(0, NB)(lambda i: prep(0, i))
    cp_x.wait()
    glu_half(0, 0, lambda i: [functools.partial(layernorm, i + 1)])
    start(gather_copies(wq_hbm, 0))
    for c in range(CB, NC):
        start(chunk_copies(c))
    wait(chunk_copies(1))
    cp_x2.wait()

    def side(i):
        return [functools.partial(layernorm, jnp.minimum(NH + i + 1, NB - 1))] + preps(1, i)

    glu_half(0, 1, side)
    start(gather_copies(wk_hbm, 1))
    cp_o.start()
    wait(chunk_copies(2))
    glu_half(1, 0, lambda i: preps(2, i))
    wait(gather_copies(wq_hbm, 0))
    for c in range(CB, NC):
        wait(chunk_copies(c))

    def side(i):
        return repacks(0, wq_v, i) + preps(3, i)

    glu_half(1, 1, side)
    start(gather_copies(wv_hbm, 0))
    wait(gather_copies(wk_hbm, 1))

    def side(i):
        return repacks(1, wk_v, i) + preps(4, i) + preps(5, i)

    glu_half(2, 0, side)
    wait(gather_copies(wv_hbm, 0))

    def side(i):
        return repacks(0, wv_v, i) + preps(6, i)

    glu_half(2, 1, side)
    cp_o.wait()
    s_v[...] = jnp.zeros_like(s_v)

    row = jax.lax.broadcasted_iota(jnp.int32, (2 * L, 2 * L), 0)
    col = jax.lax.broadcasted_iota(jnp.int32, (2 * L, 2 * L), 1)
    r_in = jnp.where(row >= L, row - L, row)
    c_in = jnp.where(col >= L, col - L, col)
    mask = ((row >= L) == (col >= L)) & ((r_in < M) | (r_in >= c_in))
    NU = H // 2
    UW = 2 * E

    def qkv(hb, u):
        return tuple(
            jnp.dot(hb, _as_bf16(w[:, u * UW:(u + 1) * UW]), preferred_element_type=_F32)
            for w in (wq_v, wk_v, wv_v))

    def stack(t):
        return jnp.concatenate([t[:, :E], t[:, E:]], axis=0).astype(_BF16)

    def scores(q, k):
        sc = jax.lax.dot_general(stack(q), stack(k), (((1,), (1,)), ((), ())),
                                 preferred_element_type=_F32) * scale
        sc = jnp.where(mask, sc, -1e9)
        e = jnp.exp(sc - jnp.max(sc, axis=-1, keepdims=True))
        return (e / jnp.sum(e, axis=-1, keepdims=True)).astype(_BF16)

    def pv(p, v):
        o = jnp.dot(p, stack(v), preferred_element_type=_F32)
        return jnp.concatenate([o[:L], o[L:]], axis=1)

    def proj(o, u):
        return jnp.dot(o.astype(_BF16), _as_bf16(wo_v[u * E:(u + 1) * E, :]),
                       preferred_element_type=_F32)

    def half(hb, fix_qkv, fix_o, fill):
        res = None
        saved = [None] * NU
        raw = qkv(hb, 0)
        prev_o = None
        for u in range(NU):
            q, k, v = fix_qkv(u, raw)
            p = scores(q, k)
            if u + 1 < NU:
                raw = qkv(hb, u + 1)
            elif prev_o is not None:
                d = proj(prev_o, u - 1)
                res = d if res is None else res + d
                prev_o = None
            fill()
            o = pv(p, v)
            if prev_o is not None:
                d = proj(prev_o, u - 1)
                res = d if res is None else res + d
            prev_o, saved[u] = fix_o(u, o)
        fill()
        fill()
        d = proj(prev_o, NU - 1)
        return res + d, saved

    def emit_out(r):
        xr = x_v[pl.ds(r, 2 * SEG), :].astype(_F32)
        gate = jax.nn.silu(gate_v[pl.ds(r, 2 * SEG), :])
        out_v[pl.ds(r, 2 * SEG), :] = (xr + s_v[...] * gate).astype(out_v.dtype)

    def out_copy(r):
        return pltpu.make_async_copy(out_v.at[pl.ds(r, 2 * SEG), :], out_hbm.at[pl.ds(r, 2 * SEG), :],
                                     sems.at[0])

    def pair_step(j, mem):
        r = pl.multiple_of(j * (2 * SEG), 2 * SEG)
        hb = jnp.concatenate([mem, xn_v[pl.ds(r, SEG + 8), :]], axis=0).astype(_BF16)
        extra = [None] * NU

        def fq_a(u, raw):
            extra[u] = tuple(t[L:] for t in raw)
            return tuple(t[:L] for t in raw)

        def fo_a(u, o):
            return o[:SEG], o[SEG:]

        def glu_all():
            for c in range(CB, NC):
                yield from glu_gen(c, r, SEG)

        gen = glu_all()
        fill = lambda: next(gen, None)
        res_a, tail_o = half(hb, fq_a, fo_a, fill)
        fill()
        fill()
        mem = res_a[:M]
        rp = pl.multiple_of(jnp.maximum(j - 1, 0) * (2 * SEG), 2 * SEG)
        emit_out(rp)
        hb = jnp.concatenate([mem, xn_v[pl.ds(r + SEG + 8, SEG - 8), :]], axis=0).astype(_BF16)

        def fq_b(u, raw):
            return tuple(jnp.concatenate([t[:M], ex, t[M:]], axis=0) for t, ex in zip(raw, extra[u]))

        def fo_b(u, o):
            return jnp.concatenate([o[:M], tail_o[u], o[M:]], axis=0), None

        res_b, _ = half(hb, fq_b, fo_b, fill)
        for _ in gen:
            pass
        s_v[:SEG - 8, :] = res_a[M:]
        s_v[SEG - 8:, :] = res_b[M:]

        @pl.when(j > 0)
        def _():
            out_copy(rp).start()

        return res_b[:M]

    jax.lax.fori_loop(0, n_seg // 2, pair_step, mem0_ref[...].astype(_F32))
    r_last = S - 2 * SEG
    emit_out(r_last)
    out_copy(r_last).start()

    pltpu.make_async_copy(out_v, out_hbm, sems.at[0]).wait()


@functools.partial(jax.jit, static_argnames=("A_seg_len",))
def pallas_recurrent_scan__memory_aug_recurrent_mem_tr__glu_gated_glu__prompt_kernel(
    A_x: jax.Array,
    A_mem0: jax.Array,
    A_Wq: jax.Array,
    A_Wk: jax.Array,
    A_Wv: jax.Array,
    A_Wo: jax.Array,
    A_seg_len: int,
    B_x: jax.Array,
    B_w_gate: jax.Array,
    B_w_up: jax.Array,
    B_w_down: jax.Array,
):
    del B_x
    B, S, D = A_x.shape
    _, H, E = A_Wq.shape
    M = A_mem0.shape[1]
    F = B_w_gate.shape[1]
    SEG = int(A_seg_len)
    assert B == 1 and S % SEG == 0

    kern = functools.partial(_kernel, S=S, D=D, H=H, E=E, M=M, SEG=SEG, F=F, MB=256, FC=512, HG=4)
    any_spec = pl.BlockSpec(memory_space=pl.ANY)
    out = pl.pallas_call(
        kern,
        out_shape=jax.ShapeDtypeStruct((S, D), A_x.dtype),
        in_specs=[any_spec, pl.BlockSpec(memory_space=pltpu.VMEM)] + [any_spec] * 7,
        out_specs=any_spec,
        scratch_shapes=[
            pltpu.VMEM((S, D), _BF16),
            pltpu.VMEM((S, D), _F32),
            pltpu.VMEM((S, D), _F32),
            pltpu.VMEM((S, D), _BF16),
            pltpu.VMEM((D // 2, H * E), _U32),
            pltpu.VMEM((D // 2, H * E), _U32),
            pltpu.VMEM((D // 2, H * E), _U32),
            pltpu.VMEM((H * E // 2, D), _U32),
            pltpu.VMEM((D // 2, F), _U32),
            pltpu.VMEM((D // 2, F), _U32),
            pltpu.VMEM((F // 2, D), _U32),
            pltpu.VMEM((2, 2, H // 2, D // 2, E), _U32),
            pltpu.VMEM((2 * SEG, D), _F32),
            pltpu.VMEM((F // 512, 5, D // 4, 512), _U32),
            pltpu.VMEM((F // 512, 5, 128, D // 2), _U32),
            pltpu.SemaphoreType.DMA((4 + F // 512,)),
        ],
        compiler_params=pltpu.CompilerParams(vmem_limit_bytes=127 * 1024 * 1024),
    )(
        A_x.reshape(S, D),
        A_mem0.reshape(M, D),
        A_Wq.reshape(D // 2, 2, H, E),
        A_Wk.reshape(D // 2, 2, H, E),
        A_Wv.reshape(D // 2, 2, H, E),
        A_Wo.reshape(H * E, D),
        B_w_gate,
        B_w_up,
        B_w_down,
    )
    return out.reshape(B, S, D)
```
